```python
import jax
import jax.numpy as jnp

def _softmax(x, axis=-1):
    return jax.nn.softmax(x, axis=axis)
def _gelu(x):
    return jax.nn.gelu(x, approximate=True)
def _silu(x):
    return jax.nn.silu(x)
def _sigmoid(x):
    return jax.nn.sigmoid(x)
def _layernorm(x, axis=-1, eps=1e-5):
    m = jnp.mean(x, axis=axis, keepdims=True)
    v = jnp.var(x, axis=axis, keepdims=True)
    return (x - m) / jnp.sqrt(v + eps)
def _scatter_add(tgt, idx, src, axis=0):
    return tgt.at[idx].add(src)
def _segment_sum(src, seg, n):
    return jax.ops.segment_sum(src, seg, n)
class _Rng:
    def __init__(self, key):
        self._k = key
    def _next(self):
        self._k, sub = jax.random.split(self._k)
        return sub
    def normal(self, shape):
        return jax.random.normal(self._next(), shape, dtype=jnp.bfloat16)
    def randint(self, lo, hi, shape):
        return jax.random.randint(self._next(), shape, lo, hi, dtype=jnp.int32)
    def uniform(self, shape, lo=0.0, hi=1.0):
        return jax.random.uniform(self._next(), shape, jnp.bfloat16, lo, hi)
    def permutation(self, n):
        return jax.random.permutation(self._next(), n)


kernel_name = 'gated_mix__sliding_local_dilated__ssm_conv_s4__prompt'

def setup_inputs():
    _rng = _Rng(jax.random.key(int.from_bytes(__import__("os").urandom(4), "little")))
    _w = (lambda a: (lambda t: t.astype(jnp.bfloat16) if jnp.issubdtype(t.dtype, jnp.floating) else t)(jnp.asarray(a)))
    def _A_setup():
        B, S, D = 1, 2048, 640
        return {
            "x": _w((lambda *s: _rng.normal(s) * 0.05)(B, S, D)),
            "wqkv": _w((lambda *s: _rng.normal(s) * 0.05)(D, 3 * D)),
            "wo": _w((lambda *s: _rng.normal(s) * 0.05)(D, D)),
        }
    _A_in = _A_setup()

    def _B_setup():
        B, L, D, N = 1, 2048, 640, 192
        A_re = -jnp.exp((lambda *s: _rng.normal(s) * 0.05)(D, N))
        A_im = jnp.pi * (lambda *s: _rng.normal(s) * 0.05)(D, N)
        B_re = (lambda *s: _rng.normal(s) * 0.05)(D, N)
        B_im = (lambda *s: _rng.normal(s) * 0.05)(D, N)
        C_re = (lambda *s: _rng.normal(s) * 0.05)(D, N)
        C_im = (lambda *s: _rng.normal(s) * 0.05)(D, N)
        log_dt = (lambda *s: _rng.normal(s) * 0.05)(D) * 0.5 - 4.0
        Dskip = (lambda *s: _rng.normal(s) * 0.05)(D)
        return {
            "u": _w((lambda *s: _rng.normal(s) * 0.05)(B, L, D)),
            "A_re": _w(A_re),
            "A_im": _w(A_im),
            "B_re": _w(B_re),
            "B_im": _w(B_im),
            "C_re": _w(C_re),
            "C_im": _w(C_im),
            "log_dt": _w(log_dt),
            "Dskip": _w(Dskip),
        }
    _B_in = _B_setup()

    return {
        "A_x": _A_in["x"],
        "A_wqkv": _A_in["wqkv"],
        "A_wo": _A_in["wo"],
        "B_u": _B_in["u"],
        "B_A_re": _B_in["A_re"],
        "B_A_im": _B_in["A_im"],
        "B_B_re": _B_in["B_re"],
        "B_B_im": _B_in["B_im"],
        "B_C_re": _B_in["C_re"],
        "B_C_im": _B_in["C_im"],
        "B_log_dt": _B_in["log_dt"],
        "B_Dskip": _B_in["Dskip"],
        "gate_w": _w((lambda *s: _rng.normal(s) * 0.05)(640)),
    }

def reference(A_x, A_wqkv, A_wo, B_u, B_A_re, B_A_im, B_B_re, B_B_im, B_C_re, B_C_im, B_log_dt, B_Dskip, gate_w):
    def _A_ref(x, wqkv, wo):
        B, S, D = x.shape
        H = 32; Dh = D // H
        W, dil = 8, 2
        qkv = (lambda x, *d: x.transpose(*d))((x @ wqkv).reshape(B, S, 3, H, Dh), 2, 0, 3, 1, 4)
        q, k, v = qkv[0], qkv[1], qkv[2]
        scale = Dh ** -0.5
        pos = jnp.arange(S)
        off = jnp.arange(W) * dil
        idx = pos[:, None] - off[None, :]
        mask = idx >= 0
        idx_c = jnp.where(mask, idx, 0).reshape(-1)
        kg = k[:, :, idx_c, :].reshape(B, H, S, W, Dh)
        vg = v[:, :, idx_c, :].reshape(B, H, S, W, Dh)
        logits = jnp.einsum("bhsd,bhswd->bhsw", q, kg) * scale
        logits = jnp.where(mask[None, None, :, :], logits, -1e9)
        attn = _softmax(logits, axis=-1)
        o = jnp.einsum("bhsw,bhswd->bhsd", attn, vg)
        return (lambda x, *d: x.transpose(*d))(o, 0, 2, 1, 3).reshape(B, S, D) @ wo

    def _B_ref(u, A_re, A_im, B_re, B_im, C_re, C_im, log_dt, Dskip):
        Bsz, L, D = u.shape
        dt = jnp.exp(log_dt)[:, None]
        A = A_re + 1j * A_im
        Bc = B_re + 1j * B_im
        Cc = C_re + 1j * C_im
        logdA = dt * A
        dB = dt * Bc
        l = (lambda x, dt: x.astype(dt))(jnp.arange(L), A_re.dtype)
        P = jnp.exp(logdA[:, :, None] * l[None, None, :])
        K = jnp.einsum("dn,dnl,dn->dl", Cc, P, dB).real
        L2 = 2 * L
        Kp = jnp.pad(K, ((0, 0), (0, L)))
        up = (lambda x, *d: x.transpose(*d))(u, 0, 2, 1)
        up = jnp.pad(up, ((0, 0), (0, 0), (0, L)))
        Kf = (lambda x, axes=(-2,-1): jnp.fft.rfft2(x.astype(jnp.float32), axes=axes))(Kp[:, None, :], axes=(-2, -1))
        Uf = (lambda x, axes=(-2,-1): jnp.fft.rfft2(x.astype(jnp.float32), axes=axes))(up[:, :, None, :], axes=(-2, -1))
        Yf = Uf * Kf[None, :, :, :]
        y = (lambda x, s, axes=(-2,-1): jnp.fft.irfft2(x, s=s, axes=axes).astype(jnp.bfloat16))(Yf, (1, L2), axes=(-2, -1))[:, :, 0, :L]
        y = (lambda x, *d: x.transpose(*d))(y, 0, 2, 1) + u * Dskip[None, None, :]
        return y

    x = A_x
    g = _sigmoid((x * gate_w).sum(-1, keepdims=True))
    a = _A_ref(x, A_wqkv, A_wo)
    b = _B_ref(x, B_A_re, B_A_im, B_B_re, B_B_im, B_C_re, B_C_im, B_log_dt, B_Dskip)
    return g * a + (1 - g) * b
```

```python
import numpy as np

import jax
import jax.numpy as jnp
import jax.experimental.pallas as pl
import jax.experimental.pallas.tpu as pltpu

S = 2048
D = 640
N = 192
H = 32
DH = D // H
WIN, DIL = 8, 2
NT = D // 128
HALO = 16
RB = 128
CB = 256
NB = S // CB
GP = 81
F32 = jnp.float32
BF16 = jnp.bfloat16

A_PAIRS = ((1, 5), (2, 6), (3, 7), (4, 8), (258, 262), (260, 264), (516, 520),
           (772, 776), (1032, 1288), (1544, 1800))
K_TILES = ((1, 3, 5, 7), (2, 4, 6, 8), (258, 260, 262, 264), (516, 520, 772, 776),
           (1032, 1288, 1544, 1800))

OFF_FE, OFF_FO, OFF_KE, OFF_KO, OFF_G, OFF_K1B, OFF_K = 0, 256, 512, 768, 1024, 1536, 2048
F_ROWS = OFF_K + 7 * 512


def _dft_tables():
    f = np.concatenate([np.arange(0, 128, 2), np.arange(1, 128, 2)]).astype(np.float64)

    def fwd(pos, freq):
        ang = -2.0 * np.pi * np.outer(freq + 0.5, pos) / (2 * CB)
        return np.concatenate([np.cos(ang), np.sin(ang)], axis=0)

    def fwd_pm(pos):
        return np.concatenate([fwd(pos, f), fwd(pos, f + 256)], axis=0)

    m = np.arange(128)
    fe, fo = fwd(2 * m, f), fwd(2 * m + 1, f)
    lane_val = [np.array([t[i % 4] + 8 * (i // 4) for i in range(128)]) for t in K_TILES]
    ke, ko = fwd(lane_val[1], f), fwd(lane_val[0], f)
    l_round = np.arange(S).astype(np.float32).astype(BF16).astype(np.int64)

    def block(delta, vals):
        out = np.zeros((512, 128))
        lane_of = {int(v): i for i, v in enumerate(vals)}
        hit = []
        for j in range(1, CB + 1):
            l = CB * delta + j
            if l < S and int(l_round[l]) in lane_of:
                out[:, lane_of[int(l_round[l])]] += fwd_pm(np.array([j]))[:, 0]
                hit.append(l)
        return out, hit

    def with_last(vals, prev):
        vals = vals.copy()
        vals[127] = prev[127]
        return vals

    k1b, hit_b = block(1, lane_val[1])
    srcs = (lane_val[2], with_last(lane_val[3], lane_val[2]), lane_val[3],
            with_last(lane_val[4], lane_val[3]), lane_val[4], lane_val[4], lane_val[4])
    blocks, covered = [], list(hit_b)
    for delta, vals in enumerate(srcs, start=1):
        mat, hit = block(delta, vals)
        blocks.append(mat)
        covered += hit
    assert sorted(covered) == list(range(CB + 1, S))
    g = np.concatenate([fe.T, fo.T], axis=0) / CB
    table = np.concatenate([fe, fo, ke, ko, g[:, :128], g[:, 128:], k1b] + blocks, axis=0)
    assert table.shape == (F_ROWS, 128)
    return table.astype(np.float32).astype(BF16)


_F_TABLE = _dft_tables()


def _cmul(a, b):
    return a[0] * b[0] - a[1] * b[1], a[0] * b[1] + a[1] * b[0]


def _csq(a):
    return a[0] * a[0] - a[1] * a[1], (a[0] + a[0]) * a[1]


def _dot(a, b):
    return jnp.dot(a, b, preferred_element_type=F32)


def _dot_nt(a, b):
    return jax.lax.dot_general(a, b, (((1,), (1,)), ((), ())), preferred_element_type=F32)


def _kernel(x_hbm, wqkv_hbm, wo_hbm, are_hbm, aim_hbm, bre_hbm, bim_hbm, cre_hbm, cim_hbm,
            ldt_ref, dskip_ref, gw_ref, f_hbm, out_hbm,
            xs, wraw, wp, wo_raw, wo_f32, wop, praw, ftab, par, wt, q_s, k_s, v_s, o_s, g_s,
            ko_s, kf_s, uf_s, yf_s, sd_s, y_s, out_s, sem_in, sem_out):
    p_hbm = (are_hbm, aim_hbm, bre_hbm, bim_hbm, cre_hbm, cim_hbm)
    p_cp = [pltpu.make_async_copy(p_hbm[i], praw.at[i], sem_in.at[i]) for i in range(6)]
    w_cp = pltpu.make_async_copy(wqkv_hbm, wraw, sem_in.at[6])
    x_cp = [pltpu.make_async_copy(x_hbm.at[:, pl.ds(128 * c, 128)], xs.at[c], sem_in.at[7 + c])
            for c in range(NT)]
    f_cp = pltpu.make_async_copy(f_hbm, ftab, sem_in.at[12])
    wo_cp = pltpu.make_async_copy(wo_hbm, wo_raw, sem_in.at[13])
    for cp in p_cp + [w_cp] + x_cp + [f_cp, wo_cp]:
        cp.start()

    lane = jax.lax.broadcasted_iota(jnp.int32, (8, 128), 1)
    sub = jax.lax.broadcasted_iota(jnp.int32, (8, 128), 0)
    lo_lane = lane < 64
    lo_sub = sub < 4

    dt_row = jnp.exp(ldt_ref[...].astype(F32)).astype(BF16).astype(F32)

    def prep_params(c):
        rows = pl.ds(128 * c, 128)
        dt = jnp.broadcast_to(dt_row[:, 128 * c:128 * (c + 1)], (128, 128)).T
        for half in range(2):
            def ld(i):
                if half == 0:
                    return praw[i, rows, 0:128].astype(F32)
                v = praw[i, rows, 128:N].astype(F32)
                return jnp.concatenate([v, v], axis=1)
            b = (dt * ld(2), dt * ld(3))
            w = _cmul((ld(4), ld(5)), b)
            for j, v in enumerate((dt * ld(0), dt * ld(1), w[0], w[1])):
                for cc in range(4):
                    par[4 * half + j, pl.ds(128 * c + cc, 32, stride=4), :] = v[32 * cc:32 * cc + 32]

    def halves(a, b):
        return (jnp.where(lo_sub, a, pltpu.roll(b, 4, 0)), jnp.where(lo_sub, pltpu.roll(a, 4, 0), b))

    def dup(a):
        r = pltpu.roll(a, 4, 0)
        return jnp.where(lo_sub, a, r), jnp.where(lo_sub, r, a)

    def kgen_unit(unit, z_lo, z_up, w_lo, w_up):
        mult, seed = [], []
        for z1, w in ((z_lo, w_lo), (z_up, w_up)):
            p = {1: z1}
            e = 1
            while e < 1024:
                p[2 * e] = _csq(p[e])
                e *= 2
            p[192] = _cmul(p[128], p[64])
            w1 = _cmul(w, p[1])
            w5 = _cmul(w1, p[4])
            w1032 = _cmul(_cmul(w, p[8]), p[1024])
            w1288 = _cmul(w1032, p[256])
            one = (jnp.ones((8, 128), F32), jnp.zeros((8, 128), F32))
            mult.append({e: tuple(zip(dup(p[e][0]), dup(p[e][1])))
                         for e in (1, 2, 16, 32, 64, 128, 192, 256, 512)})
            seed.append({name: tuple(zip(halves(a[0], b[0]), halves(a[1], b[1])))
                         for name, a, b in (("q", w1, w5), ("r", w1032, w1288), ("v", one, p[8]))})
        for grp in range(2):
            ml = {e: m[grp] for e, m in mult[0].items()}
            mu = {e: m[grp] for e, m in mult[1].items()}

            def node_l(name):
                re, im = seed[0][name][grp]
                c, s = seed[1][name][grp]
                return (re, -im), jnp.where(lo_lane, c, -s)

            def mul_l(x, e):
                (re, im), t = x
                c, s = ml[e]
                return ((re * c + im * s, im * c - re * s),
                        t * mu[e][0] - pltpu.roll(t, 64, 1) * mu[e][1])

            a15 = node_l("q")
            a26 = mul_l(a15, 1)
            a37 = mul_l(a15, 2)
            a48 = mul_l(a26, 2)
            a260 = mul_l(a48, 256)
            a1032 = node_l("r")
            left = (a15, a26, a37, a48, mul_l(a26, 256), a260, mul_l(a48, 512),
                    mul_l(a260, 512), a1032, mul_l(a1032, 512))

            def mul_r(x, e):
                (re, im), t = x
                c, s = ml[e]
                return ((re * c - im * s, im * c + re * s),
                        t * mu[e][0] + pltpu.roll(t, 64, 1) * mu[e][1])

            c, s = seed[1]["v"][grp]
            right = [(seed[0]["v"][grp], jnp.where(lo_lane, c, s))]
            right.append(mul_r(right[0], 16))
            right += [mul_r(right[0], 32), mul_r(right[1], 32)]
            for e in (64, 128, 192):
                right += [mul_r(right[j], e) for j in range(4)]

            def operand(nodes):
                cols = [jnp.concatenate([n[0][0] for n in nodes], axis=0),
                        jnp.concatenate([n[0][1] for n in nodes], axis=0),
                        jnp.concatenate([n[1] for n in nodes], axis=0)]
                return jnp.concatenate([col.astype(BF16) for col in cols], axis=1)

            ko_s[pl.ds((2 * unit + grp) * GP, 80), :] = _dot_nt(operand(left), operand(right))

    def kgen_item(item):
        r0 = pl.multiple_of(item * 16, 16)
        ld = lambda j, u: par[j, pl.ds(r0 + 8 * u, 8), :]

        def polar(rho, theta):
            mag = jnp.exp(rho)
            return mag * jnp.cos(theta), mag * jnp.sin(theta)

        up = polar(jnp.where(lo_lane, ld(4, 0), ld(4, 1)), jnp.where(lo_lane, ld(5, 0), ld(5, 1)))
        up_r = [pltpu.roll(v, 64, 1) for v in up]
        for u in range(2):
            z_lo = polar(ld(0, u), ld(1, u))
            a, b = (up, up_r) if u == 0 else (up_r, up)
            z_up = (jnp.where(lo_lane, a[0], b[0]), jnp.where(lo_lane, -a[1], b[1]))
            wi = ld(7, u)
            kgen_unit(2 * item + u, z_lo, z_up, (ld(2, u), ld(3, u)),
                      (ld(6, u), jnp.where(lo_lane, -wi, wi)))

    def prep_wqkv(m):
        w32 = wraw.bitcast(jnp.uint32)
        for r0, nr in ((0, 128), (128, 128), (192, 128)):
            wt[...] = w32[pl.ds(r0, nr), pl.ds(pl.multiple_of(m * D, 128), D)].T
            for t in range(NT):
                blk = jnp.concatenate(
                    [wt[pl.ds(4 * t + i, H, stride=DH), :] for i in range(4)], axis=0).T
                skip = 64 if r0 == 192 else 0
                wp[m * NT + t, pl.ds(2 * (r0 + skip), 2 * (nr - skip)), :] = pltpu.bitcast(
                    blk[skip:], BF16)

    def prep_wo():
        for c in range(NT):
            wo_f32[...] = wo_raw[:, 128 * c:128 * (c + 1)].astype(F32)
            wop[c] = jnp.concatenate(
                [wo_f32[pl.ds(d, H, stride=DH), :] for d in range(DH)], axis=0).astype(BF16)

    q_scale = float(DH ** -0.5 * np.log2(np.e))

    def project(r0):
        xb = jnp.concatenate([xs[c, pl.ds(r0, RB), :] for c in range(NT)], axis=1)
        for m, dst, off in ((1, k_s, HALO), (0, q_s, 0), (2, v_s, HALO)):
            w = jnp.concatenate([wp[m * NT + t] for t in range(NT)], axis=1)
            y = _dot(xb, w)
            if m == 0:
                y = y * q_scale
            for t in range(NT):
                dst[t, pl.ds(r0 + off, RB), :] = y[:, 128 * t:128 * (t + 1)]

    def gate(r0):
        acc = None
        for c in range(NT):
            p = xs[c, pl.ds(r0, RB), :].astype(F32) * gw_ref[:, 128 * c:128 * (c + 1)].astype(F32)
            acc = p if acc is None else acc + p
        g = jax.nn.sigmoid(jnp.sum(acc, axis=1, keepdims=True))
        g_s[pl.ds(r0, RB), :] = jnp.broadcast_to(g, (RB, 128))

    def attend(r0):
        for j in range(RB // 16):
            base = r0 + 16 * j
            q = [q_s[t, pl.ds(base, 16), :] for t in range(NT)]
            logits = []
            for w in range(WIN):
                rows = pl.ds(base + HALO - DIL * w, 16)
                s = q[0] * k_s[0, rows, :]
                for t in range(1, NT):
                    s = s + q[t] * k_s[t, rows, :]
                s = s + pltpu.roll(s, 64, 1)
                s = s + pltpu.roll(s, 32, 1)
                if j == 0 and w > 0:
                    pos = base + jax.lax.broadcasted_iota(jnp.int32, (16, 128), 0)
                    s = jnp.where(pos >= DIL * w, s, -1e9 * float(np.log2(np.e)))
                logits.append(s)
            mx = logits[0]
            for s in logits[1:]:
                mx = jnp.maximum(mx, s)
            p = [jnp.exp2(s - mx) for s in logits]
            den = p[0]
            for e in p[1:]:
                den = den + e
            inv = 1.0 / den
            for t in range(NT):
                acc = p[0] * v_s[t, pl.ds(base + HALO, 16), :]
                for w in range(1, WIN):
                    acc = acc + p[w] * v_s[t, pl.ds(base + HALO - DIL * w, 16), :]
                o_s[t, pl.ds(base, 16), :] = (acc * inv).astype(BF16)

    def k_tile(g0, t):
        src = {a: 8 * i + 4 * e for i, pair in enumerate(A_PAIRS) for e, a in enumerate(pair)}
        slot = jax.lax.broadcasted_iota(jnp.int32, (32, 128), 1) % 4
        parts = []
        for cc in range(4):
            acc = None
            for a4, a in enumerate(K_TILES[t]):
                v = ko_s[pl.ds(g0 * GP + src[a] + cc, 32, stride=GP), :]
                if a4 != cc:
                    v = pltpu.roll(v, (a4 - cc) % 128, 1)
                acc = v if acc is None else jnp.where(slot == a4, v, acc)
            parts.append(acc)
        return jnp.concatenate(parts, axis=0)

    def conv_tile(c):
        tiles = [k_tile(32 * c, t) for t in range(5)]
        last = jax.lax.broadcasted_iota(jnp.int32, (128, 128), 1) == 127
        t3p = jnp.where(last, tiles[2], tiles[3]).astype(BF16)
        t4p = jnp.where(last, tiles[3], tiles[4]).astype(BF16)
        tiles = [t.astype(BF16) for t in tiles]
        e = _dot_nt(ftab[pl.ds(OFF_KE, 256), :], tiles[1])
        o = _dot_nt(ftab[pl.ds(OFF_KO, 256), :], tiles[0])
        kf_s[0, 0:256, :] = e + o
        kf_s[0, 256:512, :] = e - o
        for delta, t in enumerate((tiles[2], t3p, tiles[3], t4p, tiles[4], tiles[4], tiles[4]), 1):
            y = _dot_nt(ftab[pl.ds(OFF_K + 512 * (delta - 1), 512), :], t)
            if delta == 1:
                y = y + _dot_nt(ftab[pl.ds(OFF_K1B, 512), :], tiles[1])
            kf_s[delta] = y

        x32 = xs.bitcast(jnp.uint32)
        prev = None
        for a in range(NB):
            words = x32[c, pl.ds(128 * a, 128), :]
            xe = pltpu.bitcast(words << 16, F32).astype(BF16)
            xo = pltpu.bitcast(words & jnp.uint32(0xFFFF0000), F32).astype(BF16)
            e = _dot(ftab[pl.ds(OFF_FE, 256), :], xe)
            o = _dot(ftab[pl.ds(OFF_FO, 256), :], xo)
            cur = (e + o, e - o)
            for pm in range(2):
                u = cur[pm]
                if prev is not None:
                    p = prev[pm]
                    u = jnp.concatenate([u[0:64] - p[128:192], u[64:128] + p[192:256],
                                         u[128:192] + p[0:64], u[192:256] - p[64:128]], axis=0)
                uf_s[a, pl.ds(256 * pm, 256), :] = u
            prev = cur

        for i in range(16):
            res = []
            for pm in range(2):
                re = pl.ds(256 * pm + 8 * i, 8)
                im = pl.ds(256 * pm + 128 + 8 * i, 8)
                u = [(uf_s[a, re, :], uf_s[a, im, :]) for a in range(NB)]
                acc = [None] * NB
                for delta in range(NB):
                    k = (kf_s[delta, re, :], kf_s[delta, im, :])
                    for a in range(delta, NB):
                        t = _cmul(k, u[a - delta])
                        acc[a] = t if acc[a] is None else (acc[a][0] + t[0], acc[a][1] + t[1])
                res.append(acc)
            for a in range(NB):
                for part in range(2):
                    rows = pl.ds(128 * part + 8 * i, 8)
                    yf_s[a, 0, rows, :] = res[0][a][part] + res[1][a][part]
                    yf_s[a, 1, rows, :] = res[0][a][part] - res[1][a][part]

        rows = pl.ds(pl.multiple_of(128 * c, 128), 128)
        cb = None
        for cols in (slice(0, 128), slice(128, N)):
            v = (praw[4, rows, cols].astype(F32) * praw[2, rows, cols].astype(F32)
                 - praw[5, rows, cols].astype(F32) * praw[3, rows, cols].astype(F32))
            if cb is not None:
                v = cb + jnp.concatenate([v, jnp.zeros_like(v)], axis=1)
            cb = v
        skip = sd_s[0, pl.ds(c, 1), :] + sd_s[1, pl.ds(c, 1), :] * jnp.sum(cb.T, axis=0, keepdims=True)

        for a in range(NB):
            for par_ in range(2):
                gm = jnp.concatenate([ftab[pl.ds(OFF_G + 128 * par_, 128), :],
                                      ftab[pl.ds(OFF_G + 256 + 128 * par_, 128), :]], axis=1)
                y_s[pl.ds(CB * a + par_, 128, stride=2), :] = _dot(gm, yf_s[a, par_].astype(BF16))
        for a in range(NB):
            rows = pl.ds(CB * a, CB)
            ob = jnp.concatenate([o_s[t, rows, :] for t in range(NT)], axis=1)
            att = _dot(ob, wop[c])
            g = g_s[rows, :]
            b = y_s[rows, :] + xs[c, rows, :].astype(F32) * skip
            out_s[c, rows, :] = (g * att + (1.0 - g) * b).astype(BF16)

    def out_copy(c):
        return pltpu.make_async_copy(
            out_s.at[c], out_hbm.at[:, pl.ds(pl.multiple_of(128 * c, 128), 128)], sem_out.at[c])

    for c in range(NT):
        sd_s[0, pl.ds(c, 1), :] = dskip_ref[:, 128 * c:128 * (c + 1)].astype(F32)
        sd_s[1, pl.ds(c, 1), :] = dt_row[:, 128 * c:128 * (c + 1)]
        k_s[c, 0:HALO, :] = jnp.zeros((HALO, 128), F32)
        v_s[c, 0:HALO, :] = jnp.zeros((HALO, 128), F32)
    for cp in p_cp:
        cp.wait()
    for c in range(NT):
        prep_params(c)

    @pl.loop(0, 5)
    def _(i):
        kgen_item(i)

    w_cp.wait()

    @pl.loop(0, 3)
    def _(m):
        prep_wqkv(m)
        kgen_item(5 + m)

    for cp in x_cp:
        cp.wait()

    @pl.loop(0, S // RB)
    def _(i):
        r0 = pl.multiple_of(i * RB, RB)
        project(r0)
        kgen_item(8 + 2 * i)
        kgen_item(9 + 2 * i)
        gate(r0)
        attend(r0)

    f_cp.wait()
    wo_cp.wait()
    prep_wo()

    @pl.loop(0, NT)
    def _(c):
        conv_tile(c)
        out_copy(c).start()

    for c in range(NT):
        out_copy(c).wait()


@jax.jit
def pallas_gated_mix__sliding_local_dilated__ssm_conv_s4__prompt_kernel(
    A_x: jax.Array,
    A_wqkv: jax.Array,
    A_wo: jax.Array,
    B_u: jax.Array,
    B_A_re: jax.Array,
    B_A_im: jax.Array,
    B_B_re: jax.Array,
    B_B_im: jax.Array,
    B_C_re: jax.Array,
    B_C_im: jax.Array,
    B_log_dt: jax.Array,
    B_Dskip: jax.Array,
    gate_w: jax.Array,
):
    del B_u
    hbm = pl.BlockSpec(memory_space=pl.ANY)
    vec = pl.BlockSpec(memory_space=pltpu.VMEM)
    out = pl.pallas_call(
        _kernel,
        out_shape=jax.ShapeDtypeStruct((S, D), BF16),
        in_specs=[hbm] * 9 + [vec] * 3 + [hbm],
        out_specs=hbm,
        scratch_shapes=[
            pltpu.VMEM((NT, S, 128), BF16),
            pltpu.VMEM((D, 3 * D), BF16),
            pltpu.VMEM((3 * NT, D, 128), BF16),
            pltpu.VMEM((D, D), BF16),
            pltpu.VMEM((D, 128), F32),
            pltpu.VMEM((NT, D, 128), BF16),
            pltpu.VMEM((6, D, N), BF16),
            pltpu.VMEM((F_ROWS, 128), BF16),
            pltpu.VMEM((8, D, 128), F32),
            pltpu.VMEM((D, 128), jnp.uint32),
            pltpu.VMEM((NT, S, 128), F32),
            pltpu.VMEM((NT, HALO + S, 128), F32),
            pltpu.VMEM((NT, HALO + S, 128), F32),
            pltpu.VMEM((NT, S, 128), BF16),
            pltpu.VMEM((S, 128), F32),
            pltpu.VMEM((D // 4 * GP, 128), F32),
            pltpu.VMEM((NB, 512, 128), F32),
            pltpu.VMEM((NB, 512, 128), F32),
            pltpu.VMEM((NB, 2, 256, 128), F32),
            pltpu.VMEM((2, 8, 128), F32),
            pltpu.VMEM((S, 128), F32),
            pltpu.VMEM((NT, S, 128), BF16),
            pltpu.SemaphoreType.DMA((14,)),
            pltpu.SemaphoreType.DMA((NT,)),
        ],
        compiler_params=pltpu.CompilerParams(vmem_limit_bytes=100 * 1024 * 1024),
        name="gated_mix",
    )(A_x.reshape(S, D), A_wqkv, A_wo, B_A_re, B_A_im, B_B_re, B_B_im, B_C_re, B_C_im,
      B_log_dt.reshape(1, D), B_Dskip.reshape(1, D), gate_w.reshape(1, D), _F_TABLE)
    return out.reshape(1, S, D)
```

```python
import numpy as np

import jax
import jax.numpy as jnp
import jax.experimental.pallas as pl
import jax.experimental.pallas.tpu as pltpu

S = 2048
D = 640
N = 192
H = 32
DH = D // H
WIN, DIL = 8, 2
NT = D // 128
HALO = 16
RB = 128
CB = 256
NB = S // CB
GP = 81
OB, OB_FIRST = 128, 2
PROJ_TILES = 3
UNITS = D // 8 // (S // RB)
MIX_LAG, MB = 1, 32
LINK_Q, LINK_V = (0, 1, 2, 3, 4, 5, 6), (0, 1, 2, 3, 4)
PRODUCT_GROUPS = ((7, 3), (6, 4, 0), (5, 2, 1))
F32 = jnp.float32
BF16 = jnp.bfloat16
U32 = jnp.uint32

A_PAIRS = ((1, 5), (2, 6), (3, 7), (4, 8), (258, 262), (260, 264), (516, 520),
           (772, 776), (1032, 1288), (1544, 1800))
K_TILES = ((1, 3, 5, 7), (2, 4, 6, 8), (258, 260, 262, 264), (516, 520, 772, 776),
           (1032, 1288, 1544, 1800))

OFF_FE, OFF_FO, OFF_G, OFF_K = 0, 256, 512, 1024
F_ROWS = OFF_K + 10 * 512

P_TAB = 0
P_WP = P_TAB + F_ROWS // 2
P_WO = P_WP + 3 * NT * D // 2
P_KT = P_WO + NT * D // 2
P_ROWS = P_KT + 7 * 64
P_X = 0
P_G = P_X + NT * S // 2
P_OUT = P_G + S
IO_ROWS = P_OUT + NT * S // 2


def _dft_tables():
    f = np.concatenate([np.arange(0, 128, 2), np.arange(1, 128, 2)]).astype(np.float64)

    def fwd(pos, freq):
        ang = -2.0 * np.pi * np.outer(freq + 0.5, pos) / (2 * CB)
        return np.concatenate([np.cos(ang), np.sin(ang)], axis=0)

    def fwd_pm(pos):
        return np.concatenate([fwd(pos, f), fwd(pos, f + 256)], axis=0)

    m = np.arange(128)
    fe, fo = fwd(2 * m, f), fwd(2 * m + 1, f)
    lane_val = [np.array([t[i % 8 // 2] + 32 * (i // 16) + 16 * (i % 2) + 8 * (i // 8 % 2)
                          for i in range(128)]) for t in K_TILES]
    l_round = np.arange(S).astype(np.float32).astype(BF16).astype(np.int64)

    def block(delta, vals):
        out = np.zeros((512, 128))
        lane_of = {int(v): i for i, v in enumerate(vals)}
        hit = []
        for j in range(1, CB + 1):
            l = CB * delta + j
            if l < S and int(l_round[l]) in lane_of:
                out[:, lane_of[int(l_round[l])]] += fwd_pm(np.array([j]))[:, 0]
                hit.append(l)
        return out, hit

    def with_last(vals, prev):
        vals = vals.copy()
        vals[127] = prev[127]
        return vals

    k1b, hit_b = block(1, lane_val[1])
    k0 = [block(0, lane_val[0])[0], block(0, lane_val[1])[0]]
    srcs = (lane_val[2], with_last(lane_val[3], lane_val[2]), lane_val[3],
            with_last(lane_val[4], lane_val[3]), lane_val[4], lane_val[4], lane_val[4])
    blocks, covered = [], list(hit_b)
    for delta, vals in enumerate(srcs, start=1):
        mat, hit = block(delta, vals)
        blocks.append(mat)
        covered += hit
    assert sorted(covered) == list(range(CB + 1, S))
    g = np.concatenate([fe.T, fo.T], axis=0) / CB
    order = np.concatenate([256 * (j // 2) + 64 * (j % 2) + 128 * part + np.arange(64)
                            for j in range(4) for part in range(2)])
    table = np.concatenate([fe, fo, g[:, :128], g[:, 128:]]
                           + [mat[order] for mat in k0 + [k1b] + blocks], axis=0)
    assert table.shape == (F_ROWS, 128)
    bits = table.astype(np.float32).astype(BF16).view(np.uint16).astype(np.uint32)
    return bits[0::2] | (bits[1::2] << 16)


_F_TABLE = _dft_tables()


def _cmul(a, b):
    return a[0] * b[0] - a[1] * b[1], a[0] * b[1] + a[1] * b[0]


def _csq(a):
    return a[0] * a[0] - a[1] * a[1], (a[0] + a[0]) * a[1]


def _pack_rows(a, b):
    return pltpu.pack_elementwise([a, b], packed_dtype=BF16)


def _to_bf16(words):
    return pltpu.bitcast(words, BF16)


def _to_words(v):
    return pltpu.bitcast(v.astype(BF16), U32)


def _dot(a, b):
    return jnp.dot(a, b, preferred_element_type=F32)


def _dot_nt(a, b):
    return jax.lax.dot_general(a, b, (((1,), (1,)), ((), ())), preferred_element_type=F32)


def _weave(*streams):
    done = [0] * len(streams)
    live = set(range(len(streams)))
    while live:
        i = min(live, key=lambda j: ((done[j] + 0.5) / streams[j][1], j))
        try:
            next(streams[i][0])
            done[i] += 1
        except StopIteration:
            live.remove(i)


def _chain(*gens):
    for g in gens:
        yield from g


def _kernel(x_hbm, wqkv_hbm, wo_hbm, are_hbm, aim_hbm, bre_hbm, bim_hbm, cre_hbm, cim_hbm,
            ldt_ref, dskip_ref, gw_ref, f_hbm, out_hbm,
            xs, pool, io, o_s, last_s, zero_s, wraw, wo_raw, wo_f32, praw, par, wt, qa, ka, va, qb, kb, vb,
            ko_s, uf_s, mt, sd_s, y_s, att_s, sem_in, sem_out):
    p_hbm = (are_hbm, aim_hbm, bre_hbm, bim_hbm, cre_hbm, cim_hbm)
    p_cp = [pltpu.make_async_copy(p_hbm[i], praw.at[i], sem_in.at[i]) for i in range(6)]
    w_cp = [pltpu.make_async_copy(wqkv_hbm.at[:, pl.ds(D * m, D)], wraw.at[m], sem_in.at[6 + m])
            for m in range(3)]
    x_cp = [pltpu.make_async_copy(x_hbm.at[:, pl.ds(128 * c, 128)], xs.at[c], sem_in.at[9 + c])
            for c in range(NT)]
    f_cp = pltpu.make_async_copy(f_hbm, pool.at[pl.ds(P_TAB, F_ROWS // 2)], sem_in.at[14])
    wo_cp = pltpu.make_async_copy(wo_hbm, wo_raw, sem_in.at[15])

    def table(off, rows):
        return _to_bf16(pool[pl.ds(P_TAB + off // 2, rows // 2), :])

    zero_s[0] = 0
    zero = pl.multiple_of(zero_s[0], 8)

    def link(ref, v):
        ref[0, pl.ds(HALO + RB + zero, 8), :] = v[0:8]

    def pool_rows(start, size):
        return pl.ds(start if isinstance(start, int) else pl.multiple_of(start, 8), size)

    def prep_params(c):
        cols = pl.ds(pl.multiple_of(128 * c, 128), 128)
        dt = sd_s[1, pl.ds(c, 1), :]
        ld = lambda i: praw[i, :, cols].astype(F32)
        mag, theta = jnp.exp(dt * ld(0)), dt * ld(1)
        z = (mag * jnp.cos(theta), mag * jnp.sin(theta))
        w = _cmul((ld(4), ld(5)), (dt * ld(2), dt * ld(3)))
        sd_s[0, pl.ds(c, 1), :] = sd_s[0, pl.ds(c, 1), :] + jnp.sum(w[0], axis=0, keepdims=True)
        for j, v in enumerate((z[0], z[1], w[0], w[1])):
            for half, u in enumerate((v[0:128], jnp.concatenate([v[128:N]] * 2, axis=0))):
                u = u.T
                for cc in range(4):
                    par[4 * half + j, pl.ds(128 * c + cc, 32, stride=4), :] = u[32 * cc:32 * cc + 32]

    MULTS = (1, 16, 256, 512)
    SEED0 = 2 * len(MULTS)

    def prep_powers(c):
        lo_s = jax.lax.broadcasted_iota(jnp.int32, (4, 8, 128), 1) < 4
        lo_l = jax.lax.broadcasted_iota(jnp.int32, (4, 8, 128), 2) < 64
        swap = lambda v: v if isinstance(v, float) else pltpu.roll(v, 4, 1)
        for chunk in range(4):
            rows = pl.ds(pl.multiple_of(128 * c + 32 * chunk, 32), 32)
            for half in range(2):
                def put(i, lo, hi):
                    if half and hi is lo:
                        mt[2, i, rows, :] = jnp.where(lo_s == lo_l, lo, swap(lo)).reshape(32, 128)
                        return
                    lo_r = swap(lo)
                    hi_r = lo_r if hi is lo else swap(hi)
                    g0, g1 = jnp.where(lo_s, lo, hi_r), jnp.where(lo_s, lo_r, hi)
                    if half:
                        mt[2, i, rows, :] = jnp.where(lo_l, g0, g1).reshape(32, 128)
                    else:
                        mt[0, i, rows, :] = g0.reshape(32, 128)
                        mt[1, i, rows, :] = g1.reshape(32, 128)

                ld = lambda j: par[4 * half + j, rows, :].reshape(4, 8, 128)
                p = {1: (ld(0), ld(1))}
                w = (ld(2), ld(3))
                e = 1
                while e < 1024:
                    p[2 * e] = _csq(p[e])
                    e *= 2
                for i, e in enumerate(MULTS):
                    for part in range(2):
                        put(2 * i + part, p[e][part], p[e][part])
                w1 = _cmul(w, p[1])
                w5 = _cmul(w1, p[4])
                w1032 = _cmul(_cmul(w, p[8]), p[1024])
                w1288 = _cmul(w1032, p[256])
                for i, (u, v) in enumerate(((w1, w5), (w1032, w1288))):
                    put(SEED0 + 2 * i, u[0], v[0])
                    put(SEED0 + 2 * i + 1, -u[1], -v[1])
                put(SEED0 + 4, 1.0, p[8][0])
                put(SEED0 + 5, 0.0, p[8][1])
            yield

    KGEN_STEPS = 3

    def kgen(unit):
        def powers(s):
            ld = lambda i: tuple(mt[s, i + j, pl.ds(pl.multiple_of(8 * unit, 8), 8), :] for j in range(2))
            m = {e: ld(2 * i) for i, e in enumerate(MULTS)}
            mul_conj = lambda x, e: (x[0] * m[e][0] + x[1] * m[e][1], x[1] * m[e][0] - x[0] * m[e][1])
            left = [ld(SEED0)]
            for _ in range(3):
                left.append(mul_conj(left[-1], 1))
            left += [mul_conj(left[1], 256), mul_conj(left[3], 256)]
            for _ in range(2):
                left.append(mul_conj(left[-1], 256))
            left.append(ld(SEED0 + 2))
            left.append(mul_conj(left[-1], 512))
            right = [ld(SEED0 + 4)]
            for _ in range(15):
                right.append(_cmul(right[-1], m[16]))
            return [[jnp.concatenate([_pack_rows(nodes[j][part], nodes[j + 1][part])
                                      for j in range(0, len(nodes), 2)], axis=0) for part in range(2)]
                    for nodes in (left, right)]

        upper = [(re, pltpu.roll(im, 64, 1)) for re, im in powers(2)]
        yield
        for grp in range(2):
            ops = []
            for (re, im), (ure, uim) in zip(powers(grp), upper):
                lo_l = jax.lax.broadcasted_iota(jnp.int32, re.shape, 1) < 64
                top = jnp.where(lo_l, uim, ure) if grp else jnp.where(lo_l, ure, uim)
                ops.append(jnp.concatenate([_to_bf16(v) for v in (re, im, top)], axis=1))
            ko_s[pl.ds((2 * unit + grp) * GP, 80), :] = _dot_nt(*ops)
            yield

    def kgens(first, count):
        return _chain(*[kgen(first + u) for u in range(count)]), count * KGEN_STEPS

    def prep_wqkv(m):
        for i, (r0, nr) in enumerate(((0, 128), (128, 128), (192, 128))):
            wt[i] = pltpu.bitcast(wraw[m, pl.ds(2 * r0, 2 * nr), :], U32).T
            yield
        for i, (r0, skip) in enumerate(((0, 0), (128, 0), (192, 64))):
            for t in range(NT):
                blk = jnp.concatenate(
                    [wt[i, pl.ds(4 * t + j, H, stride=DH), :] for j in range(4)], axis=0).T
                pool[pool_rows(P_WP + (m * NT + t) * (D // 2) + r0 + skip, 128 - skip), :] = blk[skip:]
            yield

    def prep_wo():
        for c in range(NT):
            wo_f32[c] = wo_raw[:, 128 * c:128 * (c + 1)].astype(F32)
            for d in range(0, DH, 2):
                v = jnp.concatenate([wo_f32[c, pl.ds(d + j, H, stride=DH), :] for j in range(2)], axis=0)
                pool[pool_rows(P_WO + c * (D // 2) + H // 2 * d, H), :] = _to_words(v)
            yield

    q_scale = float(DH ** -0.5 * np.log2(np.e))

    def project(r0, q_s, k_s, v_s):
        xb = jnp.concatenate([xs[c, pl.ds(r0, RB), :] for c in range(NT)], axis=1)
        dst = [(ref, t, off) for ref, off in ((q_s, 0), (k_s, HALO), (v_s, HALO)) for t in range(NT)]
        for j0 in range(0, 3 * NT, PROJ_TILES):
            js = range(j0, min(j0 + PROJ_TILES, 3 * NT))
            y = _dot(xb, jnp.concatenate([_to_bf16(pool[pool_rows(P_WP + j * (D // 2), D // 2), :]) for j in js], axis=1))
            for i, j in enumerate(js):
                ref, t, off = dst[j]
                v = y[:, 128 * i:128 * (i + 1)]
                ref[t, pl.ds(off, RB), :] = v * q_scale if j < NT else v
            yield

    def gate(r0):
        for j in range(RB // 32):
            rows = pl.ds(r0 + 32 * j, 32)
            acc = None
            for c in range(NT):
                xt = xs[c, rows, :]
                io[pool_rows(P_X + c * (S // 2) + r0 // 2 + 16 * j, 16), :] = pltpu.bitcast(xt, U32)
                p = xt.astype(F32) * sd_s[2, pl.ds(c, 1), :]
                acc = p if acc is None else acc + p
            g = jax.nn.sigmoid(jnp.sum(acc, axis=1, keepdims=True))
            io[pool_rows(P_G + r0 + 32 * j, 32), :] = pltpu.bitcast(jnp.broadcast_to(g, (32, 128)), U32)
            yield

    def attend(r0, q_s, k_s, v_s, first):
        for j in range(RB // 16):
            base = 16 * j
            q = [q_s[t, pl.ds(base, 16), :] for t in range(NT)]
            logits = []
            for w in range(WIN):
                rows = pl.ds(base + HALO - DIL * w, 16)
                s = q[0] * k_s[0, rows, :]
                for t in range(1, NT):
                    s = s + q[t] * k_s[t, rows, :]
                if w in LINK_Q:
                    link(k_s, s)
                s = s + pltpu.roll(s, 64, 1)
                s = s + pltpu.roll(s, 32, 1)
                if first and j == 0 and w > 0:
                    pos = r0 + jax.lax.broadcasted_iota(jnp.int32, (16, 128), 0)
                    s = jnp.where(pos >= DIL * w, s, -1e9 * float(np.log2(np.e)))
                logits.append(s)
            yield
            mx = logits[0]
            for s in logits[1:]:
                mx = jnp.maximum(mx, s)
            p = [jnp.exp2(s - mx) for s in logits]
            den = p[0]
            for e in p[1:]:
                den = den + e
            inv = 1.0 / den
            for t in range(NT):
                acc = p[0] * v_s[t, pl.ds(base + HALO, 16), :]
                for w in range(1, WIN):
                    acc = acc + p[w] * v_s[t, pl.ds(base + HALO - DIL * w, 16), :]
                if t in LINK_V:
                    link(v_s if t + 1 < NT else k_s, acc)
                o_s[t, pool_rows(r0 // 2 + base // 2, 8), :] = _to_words(acc * inv)
            yield

    def copy_halo(src, dst):
        for s_ref, d_ref in zip(src, dst):
            for t in range(NT):
                d_ref[t, 0:HALO, :] = s_ref[t, RB:RB + HALO, :]

    def x_spectrum(a, odd_f):
        for c in range(NT):
            words = pltpu.bitcast(xs[c, pl.ds(pl.multiple_of(CB * a, CB), CB), :], U32)
            xe = pltpu.bitcast(words << 16, F32).astype(BF16)
            xo = pltpu.bitcast(words & jnp.uint32(0xFFFF0000), F32).astype(BF16)
            e, o = (_dot(jnp.concatenate([table(off + 64 * odd_f, 64), table(off + 128 + 64 * odd_f, 64)],
                                         axis=0), v) for off, v in ((OFF_FE, xe), (OFF_FO, xo)))
            for pm, cur in enumerate((e + o, e - o)):
                r = 256 * pm + 64 * odd_f
                pre, pim = last_s[c, pl.ds(r, 64), :], last_s[c, pl.ds(r + 128, 64), :]
                last_s[c, pl.ds(r, 64), :] = cur[:64]
                last_s[c, pl.ds(r + 128, 64), :] = cur[64:]
                uf_s[c, a, pl.ds(r, 64), :] = cur[:64] + pim if odd_f else cur[:64] - pim
                uf_s[c, a, pl.ds(r + 128, 64), :] = cur[64:] - pre if odd_f else cur[64:] + pre
            yield

    def k_tile(g0, t):
        src = {a: 16 * (i // 2) + 8 * e + i % 2
               for i, pair in enumerate(A_PAIRS) for e, a in enumerate(pair)}
        slot = (jax.lax.broadcasted_iota(jnp.int32, (32, 128), 1) >> 1) & 3
        parts = []
        for cc in range(4):
            acc = None
            for a4, a in enumerate(K_TILES[t]):
                v = ko_s[pl.ds(g0 * GP + src[a] + 2 * cc, 32, stride=GP), :]
                if a4 != cc:
                    v = pltpu.roll(v, 2 * (a4 - cc) % 128, 1)
                acc = v if acc is None else jnp.where(slot == a4, v, acc)
            parts.append(acc)
        return jnp.concatenate(parts, axis=0)

    def k_samples(c):
        last = jax.lax.broadcasted_iota(jnp.int32, (128, 128), 1) == 127
        tiles = [k_tile(32 * c, t) for t in range(5)]
        tiles += [jnp.where(last, tiles[2], tiles[3]), jnp.where(last, tiles[3], tiles[4])]
        for t, v in enumerate(tiles):
            pool[pl.ds(P_KT + 64 * t, 64), :] = _to_words(v)

    K_TERMS = (((0, 0), (1, 1)), ((2, 1), (3, 2)), ((4, 5),), ((5, 3),), ((6, 6),),
               ((7, 4),), ((8, 4),), ((9, 4),))

    def k_spectrum(c, chunk, out):
        for delta, terms in enumerate(K_TERMS):
            f = jnp.concatenate([table(OFF_K + 512 * i + 128 * chunk, 128) for i, _ in terms], axis=1)
            kt = jnp.concatenate([_to_bf16(pool[pool_rows(P_KT + 64 * t, 64), :])
                                  for _, t in terms], axis=1)
            out.append(_dot_nt(f, kt))
            if delta % 2:
                yield

    def block_products(c, chunk, kf):
        for i in range(8):
            r = 256 * (chunk // 2) + 64 * (chunk % 2) + 8 * i
            k = [(v[8 * i:8 * i + 8], v[64 + 8 * i:72 + 8 * i]) for v in kf]
            for outs in PRODUCT_GROUPS:
                u = [(uf_s[c, a, pl.ds(r, 8), :], uf_s[c, a, pl.ds(r + 128, 8), :])
                     for a in range(max(outs) + 1)]
                for a in outs:
                    acc = _cmul(k[0], u[a])
                    for delta in range(1, a + 1):
                        t = _cmul(k[delta], u[a - delta])
                        acc = (acc[0] + t[0], acc[1] + t[1])
                    uf_s[NT, a, pl.ds(r + zero, 8), :] = acc[0]
                    uf_s[NT, a, pl.ds(r + 128 + zero, 8), :] = acc[1]
            yield

    def out_proj(c, blocks):
        for j in blocks:
            ob = jnp.concatenate(
                [_to_bf16(o_s[t, pl.ds(OB // 2 * j, OB // 2), :]) for t in range(NT)],
                axis=1)
            att_s[pl.ds(OB * j, OB), :] = _dot(ob, _to_bf16(pool[pool_rows(P_WO + c * (D // 2), D // 2), :]))
            yield

    def finish(c):
        skip = sd_s[0, pl.ds(c, 1), :]

        def inverse(a):
            yp, ym = uf_s[NT, a, 0:256, :], uf_s[NT, a, 256:512, :]
            for odd in range(2):
                gm = jnp.concatenate([table(OFF_G + 128 * odd, 128),
                                      table(OFF_G + 256 + 128 * odd, 128)], axis=1)
                y_s[a, pl.ds(odd, 128, stride=2), :] = _dot(gm, (yp - ym if odd else yp + ym).astype(BF16))

        def mix(a):
            for j in range(CB // MB):
                r = CB * a + MB * j
                half = c * (S // 2) + r // 2
                b = (y_s[a, pl.ds(MB * j, MB), :]
                     + _to_bf16(io[pool_rows(P_X + half, MB // 2), :]).astype(F32) * skip)
                g = pltpu.bitcast(io[pl.ds(P_G + r, MB), :], F32)
                io[pool_rows(P_OUT + half + zero, MB // 2), :] = _to_words(
                    b + g * (att_s[pl.ds(r, MB), :] - b))

        for a in range(NB + MIX_LAG):
            if a < NB:
                inverse(a)
            if a >= MIX_LAG:
                mix(a - MIX_LAG)

    def out_copy(c):
        src = io.bitcast(BF16).at[pl.ds(pl.multiple_of(2 * P_OUT + c * S, S), S)]
        return pltpu.make_async_copy(
            src, out_hbm.at[:, pl.ds(pl.multiple_of(128 * c, 128), 128)], sem_out.at[c])

    for cp in p_cp + w_cp:
        cp.start()
    for c in range(NT):
        row = lambda ref: ref[pl.ds(128 * c, 128)].astype(F32).reshape(1, 128)
        sd_s[0, pl.ds(c, 1), :] = row(dskip_ref)
        sd_s[1, pl.ds(c, 1), :] = jnp.exp(row(ldt_ref)).astype(BF16).astype(F32)
        sd_s[2, pl.ds(c, 1), :] = row(gw_ref)
        for ref in (qb, kb, vb, last_s):
            ref[c] = jnp.zeros(ref.shape[1:], F32)
    for cp in p_cp:
        cp.wait()
    for cp in x_cp + [f_cp]:
        cp.start()

    def prep(c):
        prep_params(c)
        yield
        yield from prep_powers(c)

    @pl.loop(0, 2)
    def _(c):
        _weave((prep(c), 5))

    for cp in w_cp:
        cp.wait()
    wo_cp.start()

    @pl.loop(0, 3)
    def _(m):
        _weave((prep(2 + m), 5), (prep_wqkv(m), 6))

    for cp in x_cp + [f_cp]:
        cp.wait()

    bufs = ((qa, ka, va), (qb, kb, vb))

    @pl.loop(0, NB)
    def _(a):
        for h in range(2):
            r0 = pl.multiple_of(a * CB + RB * h, RB)
            behind = pl.multiple_of(jnp.maximum(r0 - RB, 0), RB)
            copy_halo(bufs[1 - h][1:], bufs[h][1:])
            _weave((project(r0, *bufs[h]), 3 * NT // PROJ_TILES),
                   (attend(behind, *bufs[1 - h], h == 1), 16),
                   kgens(UNITS * (2 * a + h), UNITS), (gate(r0), 4), (x_spectrum(a, h), NT))

    wo_cp.wait()
    _weave((prep_wo(), NT), (attend(S - RB, *bufs[1], False), 16))

    @pl.loop(0, NT)
    def _(c):
        n_ob = S // OB
        _weave((out_proj(c, range(0, OB_FIRST)), 1))
        k_samples(c)
        kf = [[] for _ in range(4)]
        _weave((k_spectrum(c, 0, kf[0]), 1))
        for j in range(4):
            blocks = range(OB_FIRST + (n_ob - OB_FIRST) * j // 4, OB_FIRST + (n_ob - OB_FIRST) * (j + 1) // 4)
            streams = [(block_products(c, j, kf[j]), 8), (out_proj(c, blocks), len(blocks))]
            if j < 3:
                streams.append((k_spectrum(c, j + 1, kf[j + 1]), 4))
            _weave(*streams)
        finish(c)
        out_copy(c).start()

    for c in range(NT):
        out_copy(c).wait()


@jax.jit
def pallas_gated_mix__sliding_local_dilated__ssm_conv_s4__prompt_kernel(
    A_x: jax.Array,
    A_wqkv: jax.Array,
    A_wo: jax.Array,
    B_u: jax.Array,
    B_A_re: jax.Array,
    B_A_im: jax.Array,
    B_B_re: jax.Array,
    B_B_im: jax.Array,
    B_C_re: jax.Array,
    B_C_im: jax.Array,
    B_log_dt: jax.Array,
    B_Dskip: jax.Array,
    gate_w: jax.Array,
):
    del B_u
    hbm = pl.BlockSpec(memory_space=pl.ANY)
    vec = pl.BlockSpec(memory_space=pltpu.VMEM)
    out = pl.pallas_call(
        _kernel,
        out_shape=jax.ShapeDtypeStruct((S, D), BF16),
        in_specs=[hbm] * 9 + [vec] * 3 + [hbm],
        out_specs=hbm,
        scratch_shapes=[
            pltpu.VMEM((NT, S, 128), BF16),
            pltpu.VMEM((P_ROWS, 128), U32),
            pltpu.VMEM((IO_ROWS, 128), U32),
            pltpu.VMEM((NT, S // 2, 128), U32),
            pltpu.VMEM((NT, 512, 128), F32),
            pltpu.SMEM((1,), jnp.int32),
            pltpu.VMEM((3, D, D), BF16),
            pltpu.VMEM((D, D), BF16),
            pltpu.VMEM((NT, D, 128), F32),
            pltpu.VMEM((6, N, D), BF16),
            pltpu.VMEM((8, D, 128), F32),
            pltpu.VMEM((3, D, 128), U32),
            pltpu.VMEM((NT, RB, 128), F32),
            pltpu.VMEM((NT, HALO + RB + 8, 128), F32),
            pltpu.VMEM((NT, HALO + RB + 8, 128), F32),
            pltpu.VMEM((NT, RB, 128), F32),
            pltpu.VMEM((NT, HALO + RB + 8, 128), F32),
            pltpu.VMEM((NT, HALO + RB + 8, 128), F32),
            pltpu.VMEM((D // 4 * GP, 128), F32),
            pltpu.VMEM((NT + 1, NB, 512, 128), F32),
            pltpu.VMEM((3, 14, D, 128), F32),
            pltpu.VMEM((3, 8, 128), F32),
            pltpu.VMEM((NB, CB, 128), F32),
            pltpu.VMEM((S, 128), F32),
            pltpu.SemaphoreType.DMA((16,)),
            pltpu.SemaphoreType.DMA((NT,)),
        ],
        compiler_params=pltpu.CompilerParams(vmem_limit_bytes=100 * 1024 * 1024),
        name="gated_mix",
    )(A_x.reshape(S, D), A_wqkv, A_wo, B_A_re.T, B_A_im.T, B_B_re.T, B_B_im.T, B_C_re.T,
      B_C_im.T, B_log_dt, B_Dskip, gate_w, _F_TABLE)
    return out.reshape(1, S, D)
```

```python
import numpy as np

import jax
import jax.numpy as jnp
import jax.experimental.pallas as pl
import jax.experimental.pallas.tpu as pltpu

S = 2048
D = 640
N = 192
H = 32
DH = D // H
WIN, DIL = 8, 2
NT = D // 128
HALO = 16
RB = 128
CB = 256
NB = S // CB
GP = 81
OB_AT = (1, 2, 3, 5, 8)
OB_FIRST = OB_AT[0]
WO_ROWS, ATT_STEPS = 64, 20
EARLY_ROWS = 0
PROJ_ROWS = 128
PROJ_TILES = 3
UNITS = D // 8 // (S // RB)
UNITS_1 = 4
MIX_LAG, MB = 2, 64
PRODUCT_GROUPS = ((7,), (6, 0), (5, 1), (4, 2), (3,))
N_SEMS = 15
QP = 136
F32 = jnp.float32
BF16 = jnp.bfloat16
U32 = jnp.uint32

A_PAIRS = ((1, 5), (2, 6), (3, 7), (4, 8), (258, 262), (260, 264), (516, 520),
           (772, 776), (1032, 1288), (1544, 1800))
K_TILES = ((1, 3, 5, 7), (2, 4, 6, 8), (258, 260, 262, 264), (516, 520, 772, 776),
           (1032, 1288, 1544, 1800))

OFF_FE, OFF_FO, OFF_G, OFF_K = 0, 256, 512, 1024
F_ROWS = OFF_K + 10 * 512

P_TAB = 0
P_WP = P_TAB + F_ROWS // 2
P_WO = P_WP + 3 * NT * D // 2
P_KT = P_WO + NT * D // 2
P_PAR = P_KT + 7 * 64
P_ROWS = P_PAR + 8 * QP
P_X = 0
P_G = P_X + NT * S // 2
P_OUT = P_G + S
IO_ROWS = P_OUT + NT * S // 2


def _dft_tables():
    f = np.concatenate([np.arange(0, 128, 2), np.arange(1, 128, 2)]).astype(np.float64)

    def fwd(pos, freq):
        ang = -2.0 * np.pi * np.outer(freq + 0.5, pos) / (2 * CB)
        return np.concatenate([np.cos(ang), np.sin(ang)], axis=0)

    def fwd_pm(pos):
        return np.concatenate([fwd(pos, f), fwd(pos, f + 256)], axis=0)

    m = np.arange(128)
    fe, fo = fwd(2 * m, f), fwd(2 * m + 1, f)
    lane_val = [np.array([t[i % 8 // 2] + 32 * (i // 16) + 16 * (i % 2) + 8 * (i // 8 % 2)
                          for i in range(128)]) for t in K_TILES]
    l_round = np.arange(S).astype(np.float32).astype(BF16).astype(np.int64)

    def block(delta, vals):
        out = np.zeros((512, 128))
        lane_of = {int(v): i for i, v in enumerate(vals)}
        hit = []
        for j in range(1, CB + 1):
            l = CB * delta + j
            if l < S and int(l_round[l]) in lane_of:
                out[:, lane_of[int(l_round[l])]] += fwd_pm(np.array([j]))[:, 0]
                hit.append(l)
        return out, hit

    def with_last(vals, prev):
        vals = vals.copy()
        vals[127] = prev[127]
        return vals

    k1b, hit_b = block(1, lane_val[1])
    k0 = [block(0, lane_val[0])[0], block(0, lane_val[1])[0]]
    srcs = (lane_val[2], with_last(lane_val[3], lane_val[2]), lane_val[3],
            with_last(lane_val[4], lane_val[3]), lane_val[4], lane_val[4], lane_val[4])
    blocks, covered = [], list(hit_b)
    for delta, vals in enumerate(srcs, start=1):
        mat, hit = block(delta, vals)
        blocks.append(mat)
        covered += hit
    assert sorted(covered) == list(range(CB + 1, S))
    g = np.concatenate([fe.T, fo.T], axis=0) / CB
    order = np.concatenate([128 * part + 32 * j + np.arange(32) for j in range(4) for part in range(4)])
    table = np.concatenate([fe, fo, g[:, :128], g[:, 128:]]
                           + [mat[order] for mat in k0 + [k1b] + blocks], axis=0)
    assert table.shape == (F_ROWS, 128)
    bits = table.astype(np.float32).astype(BF16).view(np.uint16).astype(np.uint32)
    return bits[0::2] | (bits[1::2] << 16)


_F_TABLE = _dft_tables()


def _cmul(a, b):
    return a[0] * b[0] - a[1] * b[1], a[0] * b[1] + a[1] * b[0]


def _csq(a):
    return a[0] * a[0] - a[1] * a[1], (a[0] + a[0]) * a[1]


def _pack_rows(a, b):
    return pltpu.pack_elementwise([a, b], packed_dtype=BF16)


def _to_bf16(words):
    return pltpu.bitcast(words, BF16)


def _to_words(v):
    return pltpu.bitcast(v.astype(BF16), U32)


def _dot(a, b):
    return jnp.dot(a, b, preferred_element_type=F32)


def _dot_nt(a, b):
    return jax.lax.dot_general(a, b, (((1,), (1,)), ((), ())), preferred_element_type=F32)


def _weave(*streams):
    done = [0] * len(streams)
    live = set(range(len(streams)))
    while live:
        i = min(live, key=lambda j: ((done[j] + 0.5) / streams[j][1], j))
        try:
            next(streams[i][0])
            done[i] += 1
        except StopIteration:
            live.remove(i)


def _chain(*gens):
    for g in gens:
        yield from g


def _kernel(x_hbm, wqkv_hbm, wo_hbm, are_hbm, aim_hbm, bre_hbm, bim_hbm, cre_hbm, cim_hbm,
            ldt_ref, dskip_ref, gw_ref, f_hbm, out_hbm,
            xs, pool, io, o_s, wraw, wo_raw, wo_w, praw, wt, qa, ka, va, qb, kb, vb,
            ko_s, up_s, um_s, mt, sd_s, y_s, att_s, sem_in, sem_w, sem_x, sem_out):
    p_hbm = (are_hbm, aim_hbm, bre_hbm, bim_hbm, cre_hbm, cim_hbm)
    sem = iter(range(N_SEMS))

    def copy(src, dst):
        return pltpu.make_async_copy(src, dst, sem_in.at[next(sem)])

    p_cp = [[copy(ref.at[:, pl.ds(c0, nc)], praw.at[i, :, pl.ds(c0, nc)]) for i, ref in enumerate(p_hbm)]
            for c0, nc in ((0, 128), (128, D - 128))]
    wo_cp = copy(wo_hbm, wo_raw)
    f_cp = [copy(f_hbm.at[pl.ds(r0, nr)], pool.at[pl.ds(P_TAB + r0, nr)])
            for r0, nr in ((0, OFF_G // 2), (OFF_G // 2, (F_ROWS - OFF_G) // 2))]

    def w_copy(m):
        return pltpu.make_async_copy(
            wqkv_hbm.at[:, pl.ds(pl.multiple_of(D * m, 128), D)], wraw.at[m], sem_w.at[m])

    def x_copy(c):
        return pltpu.make_async_copy(
            x_hbm.at[:, pl.ds(pl.multiple_of(128 * c, 128), 128)], xs.at[c], sem_x.at[c])

    def table(off, rows):
        return _to_bf16(pool[pl.ds(P_TAB + off // 2, rows // 2), :])

    def pool_rows(start, size):
        return pl.ds(start if isinstance(start, int) else pl.multiple_of(start, 8), size)

    def prep_params(c):
        cols = pl.ds(pl.multiple_of(128 * c, 128), 128)
        dt = sd_s[1, pl.ds(c, 1), :]
        ld = lambda i: praw[i, :, cols].astype(F32)
        mag, theta = jnp.exp(dt * ld(0)), dt * ld(1)
        z = (mag * jnp.cos(theta), mag * jnp.sin(theta))
        w = _cmul((ld(4), ld(5)), (dt * ld(2), dt * ld(3)))
        sd_s[0, pl.ds(c, 1), :] = sd_s[0, pl.ds(c, 1), :] + jnp.sum(w[0], axis=0, keepdims=True)
        for j, v in enumerate((z[0], z[1], w[0], w[1])):
            for half, u in enumerate((v[0:128], jnp.concatenate([v[128:N]] * 2, axis=0))):
                u = u.T
                for cc in range(4):
                    pool[pl.ds(P_PAR + (4 * half + j) * QP + cc, 32, stride=4), :] = pltpu.bitcast(
                        u[32 * cc:32 * cc + 32], U32)

    MULTS = (1, 16, 256, 512)
    SEED0 = 2 * len(MULTS)

    def prep_powers(c):
        lo_s = jax.lax.broadcasted_iota(jnp.int32, (4, 8, 128), 1) < 4
        lo_l = jax.lax.broadcasted_iota(jnp.int32, (4, 8, 128), 2) < 64
        swap = lambda v: v if isinstance(v, float) else pltpu.roll(v, 4, 1)
        for chunk in range(4):
            rows = pl.ds(pl.multiple_of(128 * c + 32 * chunk, 32), 32)
            for half in range(2):
                def put(i, lo, hi):
                    if half and hi is lo:
                        mt[2, i, rows, :] = jnp.where(lo_s == lo_l, lo, swap(lo)).reshape(32, 128)
                        return
                    lo_r = swap(lo)
                    hi_r = lo_r if hi is lo else swap(hi)
                    g0, g1 = jnp.where(lo_s, lo, hi_r), jnp.where(lo_s, lo_r, hi)
                    if half:
                        mt[2, i, rows, :] = jnp.where(lo_l, g0, g1).reshape(32, 128)
                    else:
                        mt[0, i, rows, :] = g0.reshape(32, 128)
                        mt[1, i, rows, :] = g1.reshape(32, 128)

                ld = lambda j: pltpu.bitcast(
                    pool[pl.ds(P_PAR + (4 * half + j) * QP + 32 * chunk, 32), :], F32).reshape(4, 8, 128)
                p = {1: (ld(0), ld(1))}
                w = (ld(2), ld(3))
                e = 1
                while e < 1024:
                    p[2 * e] = _csq(p[e])
                    e *= 2
                for i, e in enumerate(MULTS):
                    for part in range(2):
                        put(2 * i + part, p[e][part], p[e][part])
                w1 = _cmul(w, p[1])
                w5 = _cmul(w1, p[4])
                w1032 = _cmul(_cmul(w, p[8]), p[1024])
                w1288 = _cmul(w1032, p[256])
                for i, (u, v) in enumerate(((w1, w5), (w1032, w1288))):
                    put(SEED0 + 2 * i, u[0], v[0])
                    put(SEED0 + 2 * i + 1, -u[1], -v[1])
                put(SEED0 + 4, 1.0, p[8][0])
                put(SEED0 + 5, 0.0, p[8][1])
            yield

    KGEN_STEPS = 3

    def kgen(unit):
        def powers(s):
            ld = lambda i: tuple(mt[s, i + j, pl.ds(pl.multiple_of(8 * unit, 8), 8), :] for j in range(2))
            m = {e: ld(2 * i) for i, e in enumerate(MULTS)}
            mul_conj = lambda x, e: (x[0] * m[e][0] + x[1] * m[e][1], x[1] * m[e][0] - x[0] * m[e][1])
            left = [ld(SEED0)]
            for _ in range(3):
                left.append(mul_conj(left[-1], 1))
            left += [mul_conj(left[1], 256), mul_conj(left[3], 256)]
            for _ in range(2):
                left.append(mul_conj(left[-1], 256))
            left.append(ld(SEED0 + 2))
            left.append(mul_conj(left[-1], 512))
            right = [ld(SEED0 + 4)]
            for _ in range(15):
                right.append(_cmul(right[-1], m[16]))
            return [[jnp.concatenate([_pack_rows(nodes[j][part], nodes[j + 1][part])
                                      for j in range(0, len(nodes), 2)], axis=0) for part in range(2)]
                    for nodes in (left, right)]

        upper = [(re, pltpu.roll(im, 64, 1)) for re, im in powers(2)]
        yield
        for grp in range(2):
            ops = []
            for (re, im), (ure, uim) in zip(powers(grp), upper):
                lo_l = jax.lax.broadcasted_iota(jnp.int32, re.shape, 1) < 64
                top = jnp.where(lo_l, uim, ure) if grp else jnp.where(lo_l, ure, uim)
                ops.append(jnp.concatenate([_to_bf16(v) for v in (re, im, top)], axis=1))
            ko_s[pl.ds((2 * unit + grp) * GP, 80), :] = _dot_nt(*ops)
            yield

    def kgens(first, count):
        return _chain(*[kgen(first + u) for u in range(count)]), count * KGEN_STEPS

    def prep_wqkv(m):
        for i, (r0, nr) in enumerate(((0, 128), (128, 128), (192, 128))):
            wt[i] = pltpu.bitcast(wraw[m, pl.ds(2 * r0, 2 * nr), :], U32).T
        yield
        for i, (r0, skip) in enumerate(((0, 0), (128, 0), (192, 64))):
            for t in range(NT):
                blk = jnp.concatenate(
                    [wt[i, pl.ds(4 * t + j, H, stride=DH), :] for j in range(4)], axis=0).T
                pool[pool_rows(P_WP + (m * NT + t) * (D // 2) + r0 + skip, 128 - skip), :] = blk[skip:]
            yield

    def prep_wo():
        hi16 = jnp.uint32(0xFFFF0000)
        for c in range(NT):
            wo_w[c] = pltpu.bitcast(wo_raw[:, 128 * c:128 * (c + 1)], U32)
            for d in range(0, DH, 2):
                even, odd = (wo_w[c, pl.ds(DH // 2 * j + d // 2, H // 2, stride=DH), :] for j in range(2))
                pool[pl.ds(P_WO + c * (D // 2) + H // 2 * d, H), :] = jnp.concatenate(
                    [(even & ~hi16) | (odd << 16), (even >> 16) | (odd & hi16)], axis=0)

    q_scale = float(DH ** -0.5 * np.log2(np.e))

    def project(r0, q_s, k_s, v_s):
        xb = jnp.concatenate([xs[c, pl.ds(r0, RB), :] for c in range(NT)], axis=1)
        dst = [(ref, t, off) for ref, off in ((q_s, 0), (k_s, HALO), (v_s, HALO)) for t in range(NT)]
        for j0 in range(0, 3 * NT, PROJ_TILES):
            js = range(j0, min(j0 + PROJ_TILES, 3 * NT))
            w = jnp.concatenate([_to_bf16(pool[pl.ds(P_WP + j * (D // 2), D // 2), :]) for j in js], axis=1)
            for m0 in range(0, RB, PROJ_ROWS):
                y = _dot(xb[m0:m0 + PROJ_ROWS], w)
                for i, j in enumerate(js):
                    ref, t, off = dst[j]
                    v = y[:, 128 * i:128 * (i + 1)]
                    ref[t, pl.ds(off + m0, PROJ_ROWS), :] = v * q_scale if j < NT else v
                yield

    def gate(r0):
        for j in range(RB // 32):
            rows = pl.ds(r0 + 32 * j, 32)
            acc = None
            for c in range(NT):
                xt = xs[c, rows, :]
                io[pool_rows(P_X + c * (S // 2) + r0 // 2 + 16 * j, 16), :] = pltpu.bitcast(xt, U32)
                p = xt.astype(F32) * sd_s[2, pl.ds(c, 1), :]
                acc = p if acc is None else acc + p
            g = jax.nn.sigmoid(jnp.sum(acc, axis=1, keepdims=True))
            io[pool_rows(P_G + r0 + 32 * j, 32), :] = pltpu.bitcast(jnp.broadcast_to(g, (32, 128)), U32)
            yield

    def attend(r0, q_s, k_s, v_s, even):
        pending = []
        for j in range(RB // 16):
            base = 16 * j
            q = [q_s[t, pl.ds(base, 16), :] for t in range(NT)]
            logits = []
            for w in range(WIN):
                rows = pl.ds(base + HALO - DIL * w, 16)
                s = q[0] * k_s[0, rows, :]
                for t in range(1, NT):
                    s = s + q[t] * k_s[t, rows, :]
                s = s + pltpu.roll(s, 64, 1)
                s = s + pltpu.roll(s, 32, 1)
                if even and j == 0 and w > 0:
                    pos = r0 + jax.lax.broadcasted_iota(jnp.int32, (16, 128), 0)
                    s = jnp.where(pos >= DIL * w, s, -1e9 * float(np.log2(np.e)))
                logits.append(s)
            yield
            mx = logits[0]
            for s in logits[1:]:
                mx = jnp.maximum(mx, s)
            p = [jnp.exp2(s - mx) for s in logits]
            den = p[0]
            for e in p[1:]:
                den = den + e
            inv = 1.0 / den
            o = []
            for t in range(NT):
                acc = p[0] * v_s[t, pl.ds(base + HALO, 16), :]
                for w in range(1, WIN):
                    acc = acc + p[w] * v_s[t, pl.ds(base + HALO - DIL * w, 16), :]
                o.append(acc * inv)
            if even and base >= RB - EARLY_ROWS:
                pending.append(jnp.concatenate([v.astype(BF16) for v in o], axis=1))
                if len(pending) == WO_ROWS // 16:
                    w = jnp.concatenate([_to_bf16(pool[pl.ds(P_WO + t * (D // 2), D // 2), :])
                                         for t in range(NT)], axis=1)
                    y = _dot(jnp.concatenate(pending, axis=0), w)
                    pending = []
                    for t in range(NT):
                        att_s[t, pool_rows(r0 // 2 + base + 16 - WO_ROWS, WO_ROWS), :] = (
                            y[:, 128 * t:128 * (t + 1)])
            else:
                for t in range(NT):
                    o_s[t, pool_rows(r0 // 2 + base // 2, 8), :] = _to_words(o[t])
            yield

    def copy_halo(src, dst):
        for s_ref, d_ref in zip(src, dst):
            for t in range(NT):
                d_ref[t, 0:HALO, :] = s_ref[t, RB:RB + HALO, :]

    uf = (up_s, um_s)

    def x_spectrum(c):
        prev = {}
        for a in range(NB):
            words = pltpu.bitcast(xs[c, pl.ds(CB * a, CB), :], U32)
            xe = pltpu.bitcast(words << 16, F32).astype(BF16)
            xo = pltpu.bitcast(words & jnp.uint32(0xFFFF0000), F32).astype(BF16)
            for odd_f in range(2):
                e, o = (_dot(jnp.concatenate([table(off + 64 * odd_f, 64), table(off + 128 + 64 * odd_f, 64)],
                                             axis=0), v) for off, v in ((OFF_FE, xe), (OFF_FO, xo)))
                for pm, cur in enumerate((e + o, e - o)):
                    re, im = cur[:64], cur[64:]
                    if a:
                        pre, pim = prev[pm, odd_f]
                        re, im = (re + pim, im - pre) if odd_f else (re - pim, im + pre)
                    prev[pm, odd_f] = cur[:64], cur[64:]
                    uf[pm][c, a, pl.ds(64 * odd_f, 64), :] = re
                    uf[pm][c, a, pl.ds(QP + 64 * odd_f, 64), :] = im
            yield

    def k_tile(g0, t):
        src = {a: 16 * (i // 2) + 8 * e + i % 2
               for i, pair in enumerate(A_PAIRS) for e, a in enumerate(pair)}
        slot = (jax.lax.broadcasted_iota(jnp.int32, (32, 128), 1) >> 1) & 3
        parts = []
        for cc in range(4):
            acc = None
            for a4, a in enumerate(K_TILES[t]):
                v = ko_s[pl.ds(g0 * GP + src[a] + 2 * cc, 32, stride=GP), :]
                if a4 != cc:
                    v = pltpu.roll(v, 2 * (a4 - cc) % 128, 1)
                acc = v if acc is None else jnp.where(slot == a4, v, acc)
            parts.append(acc)
        return jnp.concatenate(parts, axis=0)

    def k_samples(c):
        last = jax.lax.broadcasted_iota(jnp.int32, (128, 128), 1) == 127
        tiles = [k_tile(32 * c, t) for t in range(5)]
        tiles += [jnp.where(last, tiles[2], tiles[3]), jnp.where(last, tiles[3], tiles[4])]
        for t, v in enumerate(tiles):
            pool[pl.ds(P_KT + 64 * t, 64), :] = _to_words(v)

    K_TERMS = (((0, 0), (1, 1)), ((2, 1), (3, 2)), ((4, 5),), ((5, 3),), ((6, 6),),
               ((7, 4),), ((8, 4),), ((9, 4),))

    def k_spectrum(c, chunk, out):
        for delta, terms in enumerate(K_TERMS):
            f = jnp.concatenate([table(OFF_K + 512 * i + 128 * chunk, 128) for i, _ in terms], axis=1)
            kt = jnp.concatenate([_to_bf16(pool[pool_rows(P_KT + 64 * t, 64), :])
                                  for _, t in terms], axis=1)
            out.append(_dot_nt(f, kt))
            if delta % 2:
                yield

    def block_products(c, chunk, kf):
        for i in range(4):
            r = 32 * chunk + 8 * i
            for pm in range(2):
                k = [(v[64 * pm + 8 * i:][:8], v[64 * pm + 32 + 8 * i:][:8]) for v in kf]
                for outs in PRODUCT_GROUPS:
                    u = [(uf[pm][c, a, pl.ds(r, 8), :], uf[pm][c, a, pl.ds(r + QP, 8), :])
                         for a in range(max(outs) + 1)]
                    for a in outs:
                        acc = _cmul(k[0], u[a])
                        for delta in range(1, a + 1):
                            t = _cmul(k[delta], u[a - delta])
                            acc = (acc[0] + t[0], acc[1] + t[1])
                        uf[pm][NT, a, pl.ds(r, 8), :] = acc[0]
                        uf[pm][NT, a, pl.ds(r + QP, 8), :] = acc[1]
                yield

    def out_proj(c, blocks, out):
        for a in blocks:
            parts = [(CB * a, RB - EARLY_ROWS), (CB * a + RB, RB)]
            ob = jnp.concatenate(
                [jnp.concatenate([_to_bf16(o_s[t, pl.ds(r // 2, n // 2), :]) for r, n in parts if n], axis=0)
                 for t in range(NT)], axis=1)
            out.append(_dot(ob, _to_bf16(pool[pool_rows(P_WO + c * (D // 2), D // 2), :])))
            yield

    def finish(c, att_late):
        skip = sd_s[0, pl.ds(c, 1), :]

        def inverse(a):
            yp, ym = (jnp.concatenate([uf[pm][NT, a, pl.ds(QP * j, 128), :] for j in range(2)], axis=0)
                      for pm in range(2))
            for odd in range(2):
                gm = jnp.concatenate([table(OFF_G + 128 * odd, 128),
                                      table(OFF_G + 256 + 128 * odd, 128)], axis=1)
                y_s[a, pl.ds(odd, 128, stride=2), :] = _dot(gm, (yp - ym if odd else yp + ym).astype(BF16))

        def mix(a):
            for j in range(CB // MB):
                r = CB * a + MB * j
                half = c * (S // 2) + r // 2
                b = (y_s[a, pl.ds(MB * j, MB), :]
                     + _to_bf16(io[pool_rows(P_X + half, MB // 2), :]).astype(F32) * skip)
                g = pltpu.bitcast(io[pl.ds(P_G + r, MB), :], F32)
                if MB * j >= RB:
                    att = att_late[a][MB * j - EARLY_ROWS:][:MB]
                elif MB * j >= RB - EARLY_ROWS:
                    att = att_s[c, pl.ds(RB * a + MB * j, MB), :]
                else:
                    att = att_late[a][MB * j:][:MB]
                io[pool_rows(P_OUT + half, MB // 2), :] = _to_words(b + g * (att - b))

        for a in range(NB + MIX_LAG):
            if a < NB:
                inverse(a)
            if a >= MIX_LAG:
                mix(a - MIX_LAG)

    def out_copy(c):
        src = io.bitcast(BF16).at[pl.ds(pl.multiple_of(2 * P_OUT + c * S, S), S)]
        return pltpu.make_async_copy(
            src, out_hbm.at[:, pl.ds(pl.multiple_of(128 * c, 128), 128)], sem_out.at[c])

    for cp in p_cp[0] + p_cp[1] + [w_copy(0)]:
        cp.start()
    for c in range(NT):
        row = lambda ref: ref[pl.ds(128 * c, 128)].astype(F32).reshape(1, 128)
        sd_s[0, pl.ds(c, 1), :] = row(dskip_ref)
        sd_s[1, pl.ds(c, 1), :] = jnp.exp(row(ldt_ref)).astype(BF16).astype(F32)
        sd_s[2, pl.ds(c, 1), :] = row(gw_ref)
        for ref in (qb, kb, vb):
            ref[c] = jnp.zeros(ref.shape[1:], F32)

    def prep(c):
        prep_params(c)
        yield
        yield from prep_powers(c)

    for cp in p_cp[0]:
        cp.wait()

    @pl.loop(0, 2)
    def _(c):
        _weave((prep(c), 5))

        @pl.when(c == 0)
        def _():
            for cp in p_cp[1]:
                cp.wait()
            for cp in [x_copy(0), f_cp[0], w_copy(1), x_copy(1)]:
                cp.start()

    for cp in [w_copy(2), x_copy(2), x_copy(3), x_copy(4), wo_cp]:
        cp.start()
    f_cp[0].wait()

    @pl.loop(0, 3)
    def _(m):
        w_copy(m).wait()
        x_copy(m).wait()
        _weave((prep(2 + m), 5), (prep_wqkv(m), 4), (x_spectrum(m), NB))

    f_cp[1].start()
    wo_cp.wait()
    prep_wo()
    x_copy(3).wait()
    x_copy(4).wait()
    bufs = ((qa, ka, va), (qb, kb, vb))

    @pl.loop(0, NB)
    def _(a):
        for h in range(2):
            r0 = pl.multiple_of(a * CB + RB * h, RB)
            behind = pl.multiple_of(jnp.maximum(r0 - RB, RB * (1 - h)), RB)
            copy_halo(bufs[1 - h][1:], bufs[h][1:])
            _weave((project(r0, *bufs[h]), 3 * NT / PROJ_TILES * RB / PROJ_ROWS),
                   (attend(behind, *bufs[1 - h], h == 1), ATT_STEPS),
                   kgens(2 * UNITS * a + UNITS_1 * h, 2 * UNITS - UNITS_1 if h else UNITS_1), (gate(r0), 4))

    f_cp[1].wait()
    _weave((attend(S - RB, *bufs[1], False), 16), (_chain(x_spectrum(3), x_spectrum(4)), 2 * NB))

    @pl.loop(0, NT)
    def _(c):
        att = []
        _weave((out_proj(c, range(0, OB_FIRST), att), 1))
        k_samples(c)
        kf = [[] for _ in range(4)]
        _weave((k_spectrum(c, 0, kf[0]), 1))
        for j in range(4):
            blocks = range(OB_AT[j], OB_AT[j + 1])
            streams = [(block_products(c, j, kf[j]), 8), (out_proj(c, blocks, att), max(len(blocks), 1))]
            if j < 3:
                streams.append((k_spectrum(c, j + 1, kf[j + 1]), 4))
            _weave(*streams)
        finish(c, att)
        out_copy(c).start()

    for c in range(NT):
        out_copy(c).wait()


@jax.jit
def pallas_gated_mix__sliding_local_dilated__ssm_conv_s4__prompt_kernel(
    A_x: jax.Array,
    A_wqkv: jax.Array,
    A_wo: jax.Array,
    B_u: jax.Array,
    B_A_re: jax.Array,
    B_A_im: jax.Array,
    B_B_re: jax.Array,
    B_B_im: jax.Array,
    B_C_re: jax.Array,
    B_C_im: jax.Array,
    B_log_dt: jax.Array,
    B_Dskip: jax.Array,
    gate_w: jax.Array,
):
    del B_u
    hbm = pl.BlockSpec(memory_space=pl.ANY)
    vec = pl.BlockSpec(memory_space=pltpu.VMEM)
    out = pl.pallas_call(
        _kernel,
        out_shape=jax.ShapeDtypeStruct((S, D), BF16),
        in_specs=[hbm] * 9 + [vec] * 3 + [hbm],
        out_specs=hbm,
        scratch_shapes=[
            pltpu.VMEM((NT, S, 128), BF16),
            pltpu.VMEM((P_ROWS, 128), U32),
            pltpu.VMEM((IO_ROWS, 128), U32),
            pltpu.VMEM((NT, S // 2, 128), U32),
            pltpu.VMEM((3, D, D), BF16),
            pltpu.VMEM((D, D), BF16),
            pltpu.VMEM((NT, D // 2, 128), U32),
            pltpu.VMEM((6, N, D), BF16),
            pltpu.VMEM((3, D, 128), U32),
            pltpu.VMEM((NT, RB, 128), F32),
            pltpu.VMEM((NT, HALO + RB, 128), F32),
            pltpu.VMEM((NT, HALO + RB, 128), F32),
            pltpu.VMEM((NT, RB, 128), F32),
            pltpu.VMEM((NT, HALO + RB, 128), F32),
            pltpu.VMEM((NT, HALO + RB, 128), F32),
            pltpu.VMEM((D // 4 * GP, 128), F32),
            pltpu.VMEM((NT + 1, NB, 2 * QP + 8, 128), F32),
            pltpu.VMEM((NT + 1, NB, 2 * QP + 8, 128), F32),
            pltpu.VMEM((3, 14, D + 8, 128), F32),
            pltpu.VMEM((3, 8, 128), F32),
            pltpu.VMEM((NB, CB, 128), F32),
            pltpu.VMEM((NT, S // 2, 128), F32),
            pltpu.SemaphoreType.DMA((N_SEMS,)),
            pltpu.SemaphoreType.DMA((3,)),
            pltpu.SemaphoreType.DMA((NT,)),
            pltpu.SemaphoreType.DMA((NT,)),
        ],
        compiler_params=pltpu.CompilerParams(vmem_limit_bytes=100 * 1024 * 1024),
        name="gated_mix",
    )(A_x.reshape(S, D), A_wqkv, A_wo, B_A_re.T, B_A_im.T, B_B_re.T, B_B_im.T, B_C_re.T,
      B_C_im.T, B_log_dt, B_Dskip, gate_w, _F_TABLE)
    return out.reshape(1, S, D)
```

```python
import numpy as np

import jax
import jax.numpy as jnp
import jax.experimental.pallas as pl
import jax.experimental.pallas.tpu as pltpu

S = 2048
D = 640
N = 192
H = 32
DH = D // H
WIN, DIL = 8, 2
NT = D // 128
HALO = 16
RB = 128
CB = 256
NB = S // CB
GP = 81
OB_AT = (1, 2, 3, 4, 8)
OB_FIRST = OB_AT[0]
WO_ROWS, ATT_STEPS = 64, 20
EARLY_ROWS = 0
PROJ_ROWS = 128
PROJ_TILES = 3
UNITS = D // 8 // (S // RB)
UNITS_1 = 4
MIX_LAG, MB = 2, 64
PRODUCT_GROUPS = ((7,), (6, 0), (5, 1), (4, 2), (3,))
N_SEMS = 15
QP = 136
OUT_PARTS = ((0, 1536), (1536, 512))
PROJ_ORDER = (5, 6, 7, 8, 9, 0, 1, 2, 3, 4, 10, 11, 12, 13, 14)
PW = 16
F32 = jnp.float32
BF16 = jnp.bfloat16
U32 = jnp.uint32

A_PAIRS = ((1, 5), (2, 6), (3, 7), (4, 8), (258, 262), (260, 264), (516, 520),
           (772, 776), (1032, 1288), (1544, 1800))
K_TILES = ((1, 3, 5, 7), (2, 4, 6, 8), (258, 260, 262, 264), (516, 520, 772, 776),
           (1032, 1288, 1544, 1800))

OFF_FE, OFF_FO, OFF_G, OFF_K = 0, 256, 512, 1024
F_ROWS = OFF_K + 10 * 512

P_TAB = 0
P_WP = P_TAB + F_ROWS // 2
P_WO = P_WP + 3 * NT * D // 2
P_KT = P_WO + NT * D // 2
P_PAR = P_KT + 7 * 64
P_ROWS = P_PAR + 4 * QP
P_X = 0
P_G = P_X + NT * S // 2
P_OUT = P_G + S
IO_ROWS = P_OUT + NT * S // 2


def _dft_tables():
    f = np.concatenate([np.arange(0, 128, 2), np.arange(1, 128, 2)]).astype(np.float64)

    def fwd(pos, freq):
        ang = -2.0 * np.pi * np.outer(freq + 0.5, pos) / (2 * CB)
        return np.concatenate([np.cos(ang), np.sin(ang)], axis=0)

    def fwd_pm(pos):
        return np.concatenate([fwd(pos, f), fwd(pos, f + 256)], axis=0)

    m = np.arange(128)
    fe, fo = fwd(2 * m, f), fwd(2 * m + 1, f)
    lane_val = [np.array([t[i % 8 // 2] + 32 * (i // 16) + 16 * (i % 2) + 8 * (i // 8 % 2)
                          for i in range(128)]) for t in K_TILES]
    l_round = np.arange(S).astype(np.float32).astype(BF16).astype(np.int64)

    def block(delta, vals):
        out = np.zeros((512, 128))
        lane_of = {int(v): i for i, v in enumerate(vals)}
        hit = []
        for j in range(1, CB + 1):
            l = CB * delta + j
            if l < S and int(l_round[l]) in lane_of:
                out[:, lane_of[int(l_round[l])]] += fwd_pm(np.array([j]))[:, 0]
                hit.append(l)
        return out, hit

    def with_last(vals, prev):
        vals = vals.copy()
        vals[127] = prev[127]
        return vals

    k1b, hit_b = block(1, lane_val[1])
    k0 = [block(0, lane_val[0])[0], block(0, lane_val[1])[0]]
    srcs = (lane_val[2], with_last(lane_val[3], lane_val[2]), lane_val[3],
            with_last(lane_val[4], lane_val[3]), lane_val[4], lane_val[4], lane_val[4])
    blocks, covered = [], list(hit_b)
    for delta, vals in enumerate(srcs, start=1):
        mat, hit = block(delta, vals)
        blocks.append(mat)
        covered += hit
    assert sorted(covered) == list(range(CB + 1, S))
    g = np.concatenate([fe.T, fo.T], axis=0) / CB
    order = np.concatenate([128 * part + 32 * j + np.arange(32) for j in range(4) for part in range(4)])
    table = np.concatenate([fe, fo, g[:, :128], g[:, 128:]]
                           + [mat[order] for mat in k0 + [k1b] + blocks], axis=0)
    assert table.shape == (F_ROWS, 128)
    bits = table.astype(np.float32).astype(BF16).view(np.uint16).astype(np.uint32)
    return bits[0::2] | (bits[1::2] << 16)


_F_TABLE = _dft_tables()


def _cmul(a, b):
    return a[0] * b[0] - a[1] * b[1], a[0] * b[1] + a[1] * b[0]


def _csq(a):
    return a[0] * a[0] - a[1] * a[1], (a[0] + a[0]) * a[1]


def _pack_rows(a, b):
    return pltpu.pack_elementwise([a, b], packed_dtype=BF16)


def _to_bf16(words):
    return pltpu.bitcast(words, BF16)


def _to_words(v):
    return pltpu.bitcast(v.astype(BF16), U32)


def _dot(a, b):
    return jnp.dot(a, b, preferred_element_type=F32)


def _dot_nt(a, b):
    return jax.lax.dot_general(a, b, (((1,), (1,)), ((), ())), preferred_element_type=F32)


def _weave(*streams):
    done = [0] * len(streams)
    live = set(range(len(streams)))
    while live:
        i = min(live, key=lambda j: ((done[j] + 0.5) / streams[j][1], j))
        try:
            next(streams[i][0])
            done[i] += 1
        except StopIteration:
            live.remove(i)


def _chain(*gens):
    for g in gens:
        yield from g


def _kernel(x_hbm, wqkv_hbm, wo_hbm, are_hbm, aim_hbm, bre_hbm, bim_hbm, cre_hbm, cim_hbm,
            ldt_ref, dskip_ref, gw_ref, f_hbm, out_hbm,
            xs, pool, io, o_s, wraw, wo_raw, wo_w, praw, wt, qa, ka, va, qb, kb, vb,
            ko_s, up_s, um_s, mt, sd_s, y_s, att_s, sem_in, sem_w, sem_x, sem_out):
    p_hbm = (are_hbm, aim_hbm, bre_hbm, bim_hbm, cre_hbm, cim_hbm)
    sem = iter(range(N_SEMS))

    def copy(src, dst):
        return pltpu.make_async_copy(src, dst, sem_in.at[next(sem)])

    p_cp = [[copy(ref.at[:, pl.ds(c0, nc)], praw.at[i, :, pl.ds(c0, nc)]) for i, ref in enumerate(p_hbm)]
            for c0, nc in ((0, 128), (128, D - 128))]
    wo_cp = copy(wo_hbm, wo_raw)
    f_cp = [copy(f_hbm.at[pl.ds(r0, nr)], pool.at[pl.ds(P_TAB + r0, nr)])
            for r0, nr in ((0, OFF_G // 2), (OFF_G // 2, (F_ROWS - OFF_G) // 2))]

    def w_copy(m):
        return pltpu.make_async_copy(
            wqkv_hbm.at[:, pl.ds(pl.multiple_of(D * m, 128), D)], wraw.at[m], sem_w.at[m])

    def x_copy(c):
        return pltpu.make_async_copy(
            x_hbm.at[:, pl.ds(pl.multiple_of(128 * c, 128), 128)], xs.at[c], sem_x.at[c])

    def table(off, rows):
        return _to_bf16(pool[pl.ds(P_TAB + off // 2, rows // 2), :])

    def pool_rows(start, size):
        return pl.ds(start if isinstance(start, int) else pl.multiple_of(start, 8), size)

    def prep_params(c):
        cols = pl.ds(pl.multiple_of(128 * c, 128), 128)
        dt = sd_s[1, pl.ds(c, 1), :]
        ld = lambda i: praw[i, :, cols].astype(F32)
        mag, theta = jnp.exp(dt * ld(0)), dt * ld(1)
        z = (mag * jnp.cos(theta), mag * jnp.sin(theta))
        w = _cmul((ld(4), ld(5)), (dt * ld(2), dt * ld(3)))
        sd_s[0, pl.ds(c, 1), :] = sd_s[0, pl.ds(c, 1), :] + jnp.sum(w[0], axis=0, keepdims=True)
        for j, v in enumerate((z[0], z[1], w[0], w[1])):
            for half, u in enumerate((v[0:128], jnp.concatenate([v[128:N]] * 2, axis=0))):
                u = u.T
                for cc in range(4):
                    piece = u[32 * cc:32 * cc + 32]
                    if half:
                        up_s[NT, j, pl.ds(cc, 32, stride=4), :] = piece
                    else:
                        pool[pl.ds(P_PAR + j * QP + cc, 32, stride=4), :] = pltpu.bitcast(piece, U32)

    MULTS = (1, 16, 256, 512)
    SEED0 = 2 * len(MULTS)

    def prep_powers(c):
        lo_s = jax.lax.broadcasted_iota(jnp.int32, (PW // 8, 8, 128), 1) < 4
        lo_l = jax.lax.broadcasted_iota(jnp.int32, (PW // 8, 8, 128), 2) < 64
        swap = lambda v: v if isinstance(v, float) else pltpu.roll(v, 4, 1)
        for chunk in range(128 // PW):
            rows = pl.ds(pl.multiple_of(128 * c + PW * chunk, PW), PW)
            for half in range(2):
                def put(i, lo, hi):
                    if half and hi is lo:
                        mt[2, i, rows, :] = jnp.where(lo_s == lo_l, lo, swap(lo)).reshape(PW, 128)
                        return
                    lo_r = swap(lo)
                    hi_r = lo_r if hi is lo else swap(hi)
                    g0, g1 = jnp.where(lo_s, lo, hi_r), jnp.where(lo_s, lo_r, hi)
                    if half:
                        mt[2, i, rows, :] = jnp.where(lo_l, g0, g1).reshape(PW, 128)
                    else:
                        mt[0, i, rows, :] = g0.reshape(PW, 128)
                        mt[1, i, rows, :] = g1.reshape(PW, 128)

                def ld(j):
                    v = (up_s[NT, j, pl.ds(PW * chunk, PW), :] if half else
                         pltpu.bitcast(pool[pl.ds(P_PAR + j * QP + PW * chunk, PW), :], F32))
                    return v.reshape(PW // 8, 8, 128)

                p = {1: (ld(0), ld(1))}
                w = (ld(2), ld(3))
                e = 1
                while e < 1024:
                    p[2 * e] = _csq(p[e])
                    e *= 2
                for i, e in enumerate(MULTS):
                    for part in range(2):
                        put(2 * i + part, p[e][part], p[e][part])
                w1 = _cmul(w, p[1])
                w5 = _cmul(w1, p[4])
                w1032 = _cmul(_cmul(w, p[8]), p[1024])
                w1288 = _cmul(w1032, p[256])
                for i, (u, v) in enumerate(((w1, w5), (w1032, w1288))):
                    put(SEED0 + 2 * i, u[0], v[0])
                    put(SEED0 + 2 * i + 1, -u[1], -v[1])
                put(SEED0 + 4, 1.0, p[8][0])
                put(SEED0 + 5, 0.0, p[8][1])
            yield

    KGEN_STEPS = 3

    def kgen(unit):
        def powers(s):
            ld = lambda i: tuple(mt[s, i + j, pl.ds(pl.multiple_of(8 * unit, 8), 8), :] for j in range(2))
            m = {e: ld(2 * i) for i, e in enumerate(MULTS)}
            mul_conj = lambda x, e: (x[0] * m[e][0] + x[1] * m[e][1], x[1] * m[e][0] - x[0] * m[e][1])
            left = [ld(SEED0)]
            for _ in range(3):
                left.append(mul_conj(left[-1], 1))
            left += [mul_conj(left[1], 256), mul_conj(left[3], 256)]
            for _ in range(2):
                left.append(mul_conj(left[-1], 256))
            left.append(ld(SEED0 + 2))
            left.append(mul_conj(left[-1], 512))
            right = [ld(SEED0 + 4)]
            for _ in range(15):
                right.append(_cmul(right[-1], m[16]))
            return [[jnp.concatenate([_pack_rows(nodes[j][part], nodes[j + 1][part])
                                      for j in range(0, len(nodes), 2)], axis=0) for part in range(2)]
                    for nodes in (left, right)]

        upper = [(re, pltpu.roll(im, 64, 1)) for re, im in powers(2)]
        yield
        for grp in range(2):
            ops = []
            for (re, im), (ure, uim) in zip(powers(grp), upper):
                lo_l = jax.lax.broadcasted_iota(jnp.int32, re.shape, 1) < 64
                top = jnp.where(lo_l, uim, ure) if grp else jnp.where(lo_l, ure, uim)
                ops.append(jnp.concatenate([_to_bf16(v) for v in (re, im, top)], axis=1))
            ko_s[pl.ds((2 * unit + grp) * GP, 80), :] = _dot_nt(*ops)
            yield

    def kgens(first, count):
        return _chain(*[kgen(first + u) for u in range(count)]), count * KGEN_STEPS

    def prep_wqkv(m):
        for i, (r0, nr) in enumerate(((0, 128), (128, 128), (192, 128))):
            wt[i] = pltpu.bitcast(wraw[m, pl.ds(2 * r0, 2 * nr), :], U32).T
        yield
        for i, (r0, skip) in enumerate(((0, 0), (128, 0), (192, 64))):
            for t in range(NT):
                blk = jnp.concatenate(
                    [wt[i, pl.ds(4 * t + j, H, stride=DH), :] for j in range(4)], axis=0).T
                pool[pool_rows(P_WP + (m * NT + t) * (D // 2) + r0 + skip, 128 - skip), :] = blk[skip:]
            yield

    def prep_wo():
        hi16 = jnp.uint32(0xFFFF0000)
        for c in range(NT):
            wo_w[c] = pltpu.bitcast(wo_raw[:, 128 * c:128 * (c + 1)], U32)
            for d in range(0, DH, 2):
                even, odd = (wo_w[c, pl.ds(DH // 2 * j + d // 2, H // 2, stride=DH), :] for j in range(2))
                pool[pl.ds(P_WO + c * (D // 2) + H // 2 * d, H), :] = jnp.concatenate(
                    [(even & ~hi16) | (odd << 16), (even >> 16) | (odd & hi16)], axis=0)

    q_scale = float(DH ** -0.5 * np.log2(np.e))

    def project(r0, q_s, k_s, v_s):
        xb = jnp.concatenate([xs[c, pl.ds(r0, RB), :] for c in range(NT)], axis=1)
        dst = [(ref, t, off) for ref, off in ((q_s, 0), (k_s, HALO), (v_s, HALO)) for t in range(NT)]
        for j0 in range(0, 3 * NT, PROJ_TILES):
            js = PROJ_ORDER[j0:j0 + PROJ_TILES]
            w = jnp.concatenate([_to_bf16(pool[pl.ds(P_WP + j * (D // 2), D // 2), :]) for j in js], axis=1)
            for m0 in range(0, RB, PROJ_ROWS):
                y = _dot(xb[m0:m0 + PROJ_ROWS], w)
                for i, j in enumerate(js):
                    ref, t, off = dst[j]
                    v = y[:, 128 * i:128 * (i + 1)]
                    ref[t, pl.ds(off + m0, PROJ_ROWS), :] = v * q_scale if j < NT else v
                yield

    def gate(r0):
        for j in range(RB // 32):
            rows = pl.ds(r0 + 32 * j, 32)
            acc = None
            for c in range(NT):
                xt = xs[c, rows, :]
                io[pool_rows(P_X + c * (S // 2) + r0 // 2 + 16 * j, 16), :] = pltpu.bitcast(xt, U32)
                p = xt.astype(F32) * sd_s[2, pl.ds(c, 1), :]
                acc = p if acc is None else acc + p
            g = jax.nn.sigmoid(jnp.sum(acc, axis=1, keepdims=True))
            io[pool_rows(P_G + r0 + 32 * j, 32), :] = pltpu.bitcast(jnp.broadcast_to(g, (32, 128)), U32)
            yield

    def attend(r0, q_s, k_s, v_s, even):
        pending = []
        for j in range(RB // 16):
            base = 16 * j
            q = [q_s[t, pl.ds(base, 16), :] for t in range(NT)]
            logits = []
            for w in range(WIN):
                rows = pl.ds(base + HALO - DIL * w, 16)
                s = q[0] * k_s[0, rows, :]
                for t in range(1, NT):
                    s = s + q[t] * k_s[t, rows, :]
                s = s + pltpu.roll(s, 64, 1)
                s = s + pltpu.roll(s, 32, 1)
                if even and j == 0 and w > 0:
                    pos = r0 + jax.lax.broadcasted_iota(jnp.int32, (16, 128), 0)
                    s = jnp.where(pos >= DIL * w, s, -1e9 * float(np.log2(np.e)))
                logits.append(s)
            yield
            mx = logits[0]
            for s in logits[1:]:
                mx = jnp.maximum(mx, s)
            p = [jnp.exp2(s - mx) for s in logits]
            den = p[0]
            for e in p[1:]:
                den = den + e
            inv = 1.0 / den
            o = []
            for t in range(NT):
                acc = p[0] * v_s[t, pl.ds(base + HALO, 16), :]
                for w in range(1, WIN):
                    acc = acc + p[w] * v_s[t, pl.ds(base + HALO - DIL * w, 16), :]
                o.append(acc * inv)
            if even and base >= RB - EARLY_ROWS:
                pending.append(jnp.concatenate([v.astype(BF16) for v in o], axis=1))
                if len(pending) == WO_ROWS // 16:
                    w = jnp.concatenate([_to_bf16(pool[pl.ds(P_WO + t * (D // 2), D // 2), :])
                                         for t in range(NT)], axis=1)
                    y = _dot(jnp.concatenate(pending, axis=0), w)
                    pending = []
                    for t in range(NT):
                        att_s[t, pool_rows(r0 // 2 + base + 16 - WO_ROWS, WO_ROWS), :] = (
                            y[:, 128 * t:128 * (t + 1)])
            else:
                for t in range(NT):
                    o_s[t, pool_rows(r0 // 2 + base // 2, 8), :] = _to_words(o[t])
            yield

    def copy_halo(src, dst):
        for s_ref, d_ref in zip(src, dst):
            for t in range(NT):
                d_ref[t, 0:HALO, :] = s_ref[t, RB:RB + HALO, :]

    uf = (up_s, um_s)

    def x_spectrum(c):
        prev = {}
        for a in range(NB):
            words = pltpu.bitcast(xs[c, pl.ds(CB * a, CB), :], U32)
            xe = pltpu.bitcast(words << 16, F32).astype(BF16)
            xo = pltpu.bitcast(words & jnp.uint32(0xFFFF0000), F32).astype(BF16)
            for odd_f in range(2):
                e, o = (_dot(jnp.concatenate([table(off + 64 * odd_f, 64), table(off + 128 + 64 * odd_f, 64)],
                                             axis=0), v) for off, v in ((OFF_FE, xe), (OFF_FO, xo)))
                for pm, cur in enumerate((e + o, e - o)):
                    re, im = cur[:64], cur[64:]
                    if a:
                        pre, pim = prev[pm, odd_f]
                        re, im = (re + pim, im - pre) if odd_f else (re - pim, im + pre)
                    prev[pm, odd_f] = cur[:64], cur[64:]
                    uf[pm][c, a, pl.ds(64 * odd_f, 64), :] = re
                    uf[pm][c, a, pl.ds(QP + 64 * odd_f, 64), :] = im
            yield

    def k_tile(g0, t):
        src = {a: 16 * (i // 2) + 8 * e + i % 2
               for i, pair in enumerate(A_PAIRS) for e, a in enumerate(pair)}
        slot = (jax.lax.broadcasted_iota(jnp.int32, (32, 128), 1) >> 1) & 3
        parts = []
        for cc in range(4):
            acc = None
            for a4, a in enumerate(K_TILES[t]):
                v = ko_s[pl.ds(g0 * GP + src[a] + 2 * cc, 32, stride=GP), :]
                if a4 != cc:
                    v = pltpu.roll(v, 2 * (a4 - cc) % 128, 1)
                acc = v if acc is None else jnp.where(slot == a4, v, acc)
            parts.append(acc)
        return jnp.concatenate(parts, axis=0)

    def k_samples(c):
        last = jax.lax.broadcasted_iota(jnp.int32, (128, 128), 1) == 127
        tiles = [k_tile(32 * c, t) for t in range(5)]
        tiles += [jnp.where(last, tiles[2], tiles[3]), jnp.where(last, tiles[3], tiles[4])]
        for t, v in enumerate(tiles):
            pool[pl.ds(P_KT + 64 * t, 64), :] = _to_words(v)

    K_TERMS = (((0, 0), (1, 1)), ((2, 1), (3, 2)), ((4, 5),), ((5, 3),), ((6, 6),),
               ((7, 4),), ((8, 4),), ((9, 4),))

    def k_spectrum(c, chunk, out):
        for delta, terms in enumerate(K_TERMS):
            f = jnp.concatenate([table(OFF_K + 512 * i + 128 * chunk, 128) for i, _ in terms], axis=1)
            kt = jnp.concatenate([_to_bf16(pool[pool_rows(P_KT + 64 * t, 64), :])
                                  for _, t in terms], axis=1)
            out.append(_dot_nt(f, kt))
            if delta % 2:
                yield

    def block_products(c, chunk, kf):
        for i in range(4):
            r = 32 * chunk + 8 * i
            for pm in range(2):
                k = [(v[64 * pm + 8 * i:][:8], v[64 * pm + 32 + 8 * i:][:8]) for v in kf]
                k = [(p, q - p, p + q) for p, q in k]
                for outs in PRODUCT_GROUPS:
                    u = [(uf[pm][c, a, pl.ds(r, 8), :], uf[pm][c, a, pl.ds(r + QP, 8), :])
                         for a in range(max(outs) + 1)]
                    u = [(p + q, p, q) for p, q in u]
                    for a in outs:
                        acc = [x * y for x, y in zip(k[0], u[a])]
                        for delta in range(1, a + 1):
                            acc = [z + x * y for x, y, z in zip(k[delta], u[a - delta], acc)]
                        acc = (acc[0] - acc[2], acc[0] + acc[1])
                        uf[pm][NT, a, pl.ds(r, 8), :] = acc[0]
                        uf[pm][NT, a, pl.ds(r + QP, 8), :] = acc[1]
                yield

    def out_proj(c, blocks, out):
        for a in blocks:
            parts = [(CB * a, RB - EARLY_ROWS), (CB * a + RB, RB)]
            ob = jnp.concatenate(
                [jnp.concatenate([_to_bf16(o_s[t, pl.ds(r // 2, n // 2), :]) for r, n in parts if n], axis=0)
                 for t in range(NT)], axis=1)
            out.append(_dot(ob, _to_bf16(pool[pool_rows(P_WO + c * (D // 2), D // 2), :])))
            yield

    def finish(c, att_late):
        skip = sd_s[0, pl.ds(c, 1), :]

        def inverse(a):
            yp, ym = (jnp.concatenate([uf[pm][NT, a, pl.ds(QP * j, 128), :] for j in range(2)], axis=0)
                      for pm in range(2))
            for odd in range(2):
                gm = jnp.concatenate([table(OFF_G + 128 * odd, 128),
                                      table(OFF_G + 256 + 128 * odd, 128)], axis=1)
                y_s[a, pl.ds(odd, 128, stride=2), :] = _dot(gm, (yp - ym if odd else yp + ym).astype(BF16))

        def mix(a):
            for j in range(CB // MB):
                r = CB * a + MB * j
                half = c * (S // 2) + r // 2
                b = (y_s[a, pl.ds(MB * j, MB), :]
                     + _to_bf16(io[pool_rows(P_X + half, MB // 2), :]).astype(F32) * skip)
                g = pltpu.bitcast(io[pl.ds(P_G + r, MB), :], F32)
                if MB * j >= RB:
                    att = att_late[a][MB * j - EARLY_ROWS:][:MB]
                elif MB * j >= RB - EARLY_ROWS:
                    att = att_s[c, pl.ds(RB * a + MB * j, MB), :]
                else:
                    att = att_late[a][MB * j:][:MB]
                io[pool_rows(P_OUT + half, MB // 2), :] = _to_words(b + g * (att - b))

        for a in range(NB + MIX_LAG):
            if a < NB:
                inverse(a)
            if a >= MIX_LAG:
                mix(a - MIX_LAG)
                for part, (r0, nr) in enumerate(OUT_PARTS):
                    if r0 + nr == CB * (a - MIX_LAG + 1):
                        out_copy(c, part).start()

    def out_copy(c, part):
        r0, nr = OUT_PARTS[part]
        src = io.bitcast(BF16).at[pl.ds(pl.multiple_of(2 * P_OUT + c * S + r0, CB), nr)]
        dst = out_hbm.at[pl.ds(r0, nr), pl.ds(pl.multiple_of(128 * c, 128), 128)]
        return pltpu.make_async_copy(src, dst, sem_out.at[len(OUT_PARTS) * c + part])

    for cp in p_cp[0] + p_cp[1] + [w_copy(0)]:
        cp.start()
    for c in range(NT):
        row = lambda ref: ref[pl.ds(128 * c, 128)].astype(F32).reshape(1, 128)
        sd_s[0, pl.ds(c, 1), :] = row(dskip_ref)
        sd_s[1, pl.ds(c, 1), :] = jnp.exp(row(ldt_ref)).astype(BF16).astype(F32)
        sd_s[2, pl.ds(c, 1), :] = row(gw_ref)
        for ref in (qb, kb, vb):
            ref[c] = jnp.zeros(ref.shape[1:], F32)

    def prep(c):
        prep_params(c)
        yield
        yield from prep_powers(c)

    for cp in p_cp[0]:
        cp.wait()

    @pl.loop(0, 2)
    def _(c):
        _weave((prep(c), 5))

        @pl.when(c == 0)
        def _():
            for cp in p_cp[1]:
                cp.wait()
            for cp in [x_copy(0), f_cp[0], w_copy(1), x_copy(1)]:
                cp.start()

    for cp in [w_copy(2), x_copy(2), x_copy(3), x_copy(4), wo_cp]:
        cp.start()
    f_cp[0].wait()

    @pl.loop(0, 3)
    def _(m):
        w_copy(m).wait()
        x_copy(m).wait()
        _weave((prep_wqkv(m), 4), (x_spectrum(m), NB))
        _weave((prep(2 + m), 5))

    f_cp[1].start()
    wo_cp.wait()
    prep_wo()
    x_copy(3).wait()
    x_copy(4).wait()
    bufs = ((qa, ka, va), (qb, kb, vb))

    @pl.loop(0, NB)
    def _(a):
        for h in range(2):
            r0 = pl.multiple_of(a * CB + RB * h, RB)
            behind = pl.multiple_of(jnp.maximum(r0 - RB, RB * (1 - h)), RB)
            copy_halo(bufs[1 - h][1:], bufs[h][1:])
            _weave((project(r0, *bufs[h]), 3 * NT / PROJ_TILES * RB / PROJ_ROWS),
                   (attend(behind, *bufs[1 - h], h == 1), ATT_STEPS),
                   kgens(2 * UNITS * a + UNITS_1 * h, 2 * UNITS - UNITS_1 if h else UNITS_1), (gate(r0), 4))

    f_cp[1].wait()
    _weave((attend(S - RB, *bufs[1], False), 16), (_chain(x_spectrum(3), x_spectrum(4)), 2 * NB))

    @pl.loop(0, NT)
    def _(c):
        att = []
        _weave((out_proj(c, range(0, OB_FIRST), att), 1))
        k_samples(c)
        kf = [[] for _ in range(4)]
        _weave((k_spectrum(c, 0, kf[0]), 1))
        for j in range(4):
            blocks = range(OB_AT[j], OB_AT[j + 1])
            streams = [(block_products(c, j, kf[j]), 8), (out_proj(c, blocks, att), max(len(blocks), 1))]
            if j < 3:
                streams.append((k_spectrum(c, j + 1, kf[j + 1]), 4))
            _weave(*streams)
        finish(c, att)

    for c in range(NT):
        for part in range(len(OUT_PARTS)):
            out_copy(c, part).wait()


@jax.jit
def pallas_gated_mix__sliding_local_dilated__ssm_conv_s4__prompt_kernel(
    A_x: jax.Array,
    A_wqkv: jax.Array,
    A_wo: jax.Array,
    B_u: jax.Array,
    B_A_re: jax.Array,
    B_A_im: jax.Array,
    B_B_re: jax.Array,
    B_B_im: jax.Array,
    B_C_re: jax.Array,
    B_C_im: jax.Array,
    B_log_dt: jax.Array,
    B_Dskip: jax.Array,
    gate_w: jax.Array,
):
    del B_u
    hbm = pl.BlockSpec(memory_space=pl.ANY)
    vec = pl.BlockSpec(memory_space=pltpu.VMEM)
    out = pl.pallas_call(
        _kernel,
        out_shape=jax.ShapeDtypeStruct((S, D), BF16),
        in_specs=[hbm] * 9 + [vec] * 3 + [hbm],
        out_specs=hbm,
        scratch_shapes=[
            pltpu.VMEM((NT, S, 128), BF16),
            pltpu.VMEM((P_ROWS, 128), U32),
            pltpu.VMEM((IO_ROWS, 128), U32),
            pltpu.VMEM((NT, S // 2, 128), U32),
            pltpu.VMEM((3, D, D), BF16),
            pltpu.VMEM((D, D), BF16),
            pltpu.VMEM((NT, D // 2, 128), U32),
            pltpu.VMEM((6, N, D), BF16),
            pltpu.VMEM((3, D, 128), U32),
            pltpu.VMEM((NT, RB, 128), F32),
            pltpu.VMEM((NT, HALO + RB, 128), F32),
            pltpu.VMEM((NT, HALO + RB, 128), F32),
            pltpu.VMEM((NT, RB, 128), F32),
            pltpu.VMEM((NT, HALO + RB, 128), F32),
            pltpu.VMEM((NT, HALO + RB, 128), F32),
            pltpu.VMEM((D // 4 * GP, 128), F32),
            pltpu.VMEM((NT + 1, NB, 2 * QP + 8, 128), F32),
            pltpu.VMEM((NT + 1, NB, 2 * QP + 8, 128), F32),
            pltpu.VMEM((3, 14, D + 8, 128), F32),
            pltpu.VMEM((3, 8, 128), F32),
            pltpu.VMEM((NB, CB, 128), F32),
            pltpu.VMEM((NT, S // 2, 128), F32),
            pltpu.SemaphoreType.DMA((N_SEMS,)),
            pltpu.SemaphoreType.DMA((3,)),
            pltpu.SemaphoreType.DMA((NT,)),
            pltpu.SemaphoreType.DMA((len(OUT_PARTS) * NT,)),
        ],
        compiler_params=pltpu.CompilerParams(vmem_limit_bytes=100 * 1024 * 1024),
        name="gated_mix",
    )(A_x.reshape(S, D), A_wqkv, A_wo, B_A_re.T, B_A_im.T, B_B_re.T, B_B_im.T, B_C_re.T,
      B_C_im.T, B_log_dt, B_Dskip, gate_w, _F_TABLE)
    return out.reshape(1, S, D)
```

```python
import numpy as np

import jax
import jax.numpy as jnp
import jax.experimental.pallas as pl
import jax.experimental.pallas.tpu as pltpu

S = 2048
D = 640
N = 192
H = 32
DH = D // H
WIN, DIL = 8, 2
NT = D // 128
HALO = 16
RB = 128
CB = 256
NB = S // CB
GP = 81
QP = 136
PW = 16
UNITS = D // 8 // (S // RB)
N_SEMS = 15
PROJ_TILES = 3
PROJ_ORDER = (0, 5, 1, 6, 2, 7, 3, 8, 4, 9, 10, 11, 12, 13, 14)
UNITS_1, ATT_STEPS = 4, 20
OB_AT = (1, 2, 3, 4, 8)
PRODUCT_GROUPS = ((7,), (6,), (5, 0), (4, 1), (3, 2))
MIX_LAG, MB = 1, 64
OUT_PARTS = ((0, 1024), (1024, 768), (1792, 256))
F32 = jnp.float32
BF16 = jnp.bfloat16
U32 = jnp.uint32

A_PAIRS = ((1, 5), (2, 6), (3, 7), (4, 8), (258, 262), (260, 264), (516, 520),
           (772, 776), (1032, 1288), (1544, 1800))
K_TILES = ((1, 3, 5, 7), (2, 4, 6, 8), (258, 260, 262, 264), (516, 520, 772, 776),
           (1032, 1288, 1544, 1800))

OFF_FE, OFF_FO, OFF_G, OFF_K = 0, 256, 512, 1024
F_ROWS = OFF_K + 10 * 512

P_TAB = 0
P_WP = P_TAB + F_ROWS // 2
P_WO = P_WP + 3 * NT * D // 2
P_KT = P_WO + NT * D // 2
P_PAR = P_KT + 7 * 64
P_ROWS = P_PAR + 4 * QP
P_X = 0
P_G = P_X + NT * S // 2
P_OUT = P_G + S
IO_ROWS = P_OUT + NT * S // 2


def _dft_tables():
    f = np.concatenate([np.arange(0, 128, 2), np.arange(1, 128, 2)]).astype(np.float64)

    def fwd(pos, freq):
        ang = -2.0 * np.pi * np.outer(freq + 0.5, pos) / (2 * CB)
        return np.concatenate([np.cos(ang), np.sin(ang)], axis=0)

    def fwd_pm(pos):
        return np.concatenate([fwd(pos, f), fwd(pos, f + 256)], axis=0)

    m = np.arange(128)
    fe, fo = fwd(2 * m, f), fwd(2 * m + 1, f)
    lane_val = [np.array([t[i % 8 // 2] + 32 * (i // 16) + 16 * (i % 2) + 8 * (i // 8 % 2)
                          for i in range(128)]) for t in K_TILES]
    l_round = np.arange(S).astype(np.float32).astype(BF16).astype(np.int64)

    def block(delta, vals):
        out = np.zeros((512, 128))
        lane_of = {int(v): i for i, v in enumerate(vals)}
        hit = []
        for j in range(1, CB + 1):
            l = CB * delta + j
            if l < S and int(l_round[l]) in lane_of:
                out[:, lane_of[int(l_round[l])]] += fwd_pm(np.array([j]))[:, 0]
                hit.append(l)
        return out, hit

    def with_last(vals, prev):
        vals = vals.copy()
        vals[127] = prev[127]
        return vals

    k1b, hit_b = block(1, lane_val[1])
    k0 = [block(0, lane_val[0])[0], block(0, lane_val[1])[0]]
    srcs = (lane_val[2], with_last(lane_val[3], lane_val[2]), lane_val[3],
            with_last(lane_val[4], lane_val[3]), lane_val[4], lane_val[4], lane_val[4])
    blocks, covered = [], list(hit_b)
    for delta, vals in enumerate(srcs, start=1):
        mat, hit = block(delta, vals)
        blocks.append(mat)
        covered += hit
    assert sorted(covered) == list(range(CB + 1, S))
    g = np.concatenate([fe.T, fo.T], axis=0) / CB
    order = np.concatenate([128 * part + 32 * j + np.arange(32) for j in range(4) for part in range(4)])
    table = np.concatenate([fe, fo, g[:, :128], g[:, 128:]]
                           + [mat[order] for mat in k0 + [k1b] + blocks], axis=0)
    assert table.shape == (F_ROWS, 128)
    bits = table.astype(np.float32).astype(BF16).view(np.uint16).astype(np.uint32)
    return bits[0::2] | (bits[1::2] << 16)


_F_TABLE = _dft_tables()


def _cmul(a, b):
    return a[0] * b[0] - a[1] * b[1], a[0] * b[1] + a[1] * b[0]


def _csq(a):
    return a[0] * a[0] - a[1] * a[1], (a[0] + a[0]) * a[1]


def _pack_rows(a, b):
    return pltpu.pack_elementwise([a, b], packed_dtype=BF16)


def _to_bf16(words):
    return pltpu.bitcast(words, BF16)


def _to_words(v):
    return pltpu.bitcast(v.astype(BF16), U32)


def _dot(a, b):
    return jnp.dot(a, b, preferred_element_type=F32)


def _dot_nt(a, b):
    return jax.lax.dot_general(a, b, (((1,), (1,)), ((), ())), preferred_element_type=F32)


def _weave(*streams):
    done = [0] * len(streams)
    live = set(range(len(streams)))
    while live:
        i = min(live, key=lambda j: ((done[j] + 0.5) / streams[j][1], j))
        try:
            next(streams[i][0])
            done[i] += 1
        except StopIteration:
            live.remove(i)


def _chain(*gens):
    for g in gens:
        yield from g


def _kernel(x_hbm, wqkv_hbm, wo_hbm, are_hbm, aim_hbm, bre_hbm, bim_hbm, cre_hbm, cim_hbm,
            ldt_ref, dskip_ref, gw_ref, f_hbm, out_hbm,
            xs, pool, io, o_s, wraw, wo_raw, wo_w, praw, wt, qa, ka, va, qb, kb, vb,
            ko_s, up_s, um_s, mt, sd_s, y_s, sem_in, sem_w, sem_x, sem_out):
    p_hbm = (are_hbm, aim_hbm, bre_hbm, bim_hbm, cre_hbm, cim_hbm)
    sem = iter(range(N_SEMS))

    def copy(src, dst):
        return pltpu.make_async_copy(src, dst, sem_in.at[next(sem)])

    p_cp = [[copy(ref.at[:, pl.ds(c0, nc)], praw.at[i, :, pl.ds(c0, nc)]) for i, ref in enumerate(p_hbm)]
            for c0, nc in ((0, 128), (128, D - 128))]
    wo_cp = copy(wo_hbm, wo_raw)
    f_cp = [copy(f_hbm.at[pl.ds(r0, nr)], pool.at[pl.ds(P_TAB + r0, nr)])
            for r0, nr in ((0, OFF_G // 2), (OFF_G // 2, (F_ROWS - OFF_G) // 2))]

    def w_copy(m):
        return pltpu.make_async_copy(
            wqkv_hbm.at[:, pl.ds(pl.multiple_of(D * m, 128), D)], wraw.at[m], sem_w.at[m])

    def x_copy(c):
        return pltpu.make_async_copy(
            x_hbm.at[:, pl.ds(pl.multiple_of(128 * c, 128), 128)], xs.at[c], sem_x.at[c])

    def table(off, rows):
        return _to_bf16(pool[pl.ds(P_TAB + off // 2, rows // 2), :])

    def pool_rows(start, size):
        return pl.ds(start if isinstance(start, int) else pl.multiple_of(start, 8), size)

    def prep_params(c):
        cols = pl.ds(pl.multiple_of(128 * c, 128), 128)
        dt = sd_s[1, pl.ds(c, 1), :]
        ld = lambda i: praw[i, :, cols].astype(F32)
        mag, theta = jnp.exp(dt * ld(0)), dt * ld(1)
        z = (mag * jnp.cos(theta), mag * jnp.sin(theta))
        w = _cmul((ld(4), ld(5)), (dt * ld(2), dt * ld(3)))
        sd_s[0, pl.ds(c, 1), :] = sd_s[0, pl.ds(c, 1), :] + jnp.sum(w[0], axis=0, keepdims=True)
        for j, v in enumerate((z[0], z[1], w[0], w[1])):
            for half, u in enumerate((v[0:128], jnp.concatenate([v[128:N]] * 2, axis=0))):
                u = u.T
                for cc in range(4):
                    piece = u[32 * cc:32 * cc + 32]
                    if half:
                        up_s[NT, j, pl.ds(cc, 32, stride=4), :] = piece
                    else:
                        pool[pl.ds(P_PAR + j * QP + cc, 32, stride=4), :] = pltpu.bitcast(piece, U32)

    MULTS = (1, 16, 256, 512)
    SEED0 = 2 * len(MULTS)

    def prep_powers(c):
        lo_s = jax.lax.broadcasted_iota(jnp.int32, (PW // 8, 8, 128), 1) < 4
        lo_l = jax.lax.broadcasted_iota(jnp.int32, (PW // 8, 8, 128), 2) < 64
        swap = lambda v: v if isinstance(v, float) else pltpu.roll(v, 4, 1)
        for chunk in range(128 // PW):
            rows = pl.ds(pl.multiple_of(128 * c + PW * chunk, PW), PW)
            for half in range(2):
                def put(i, lo, hi):
                    if half and hi is lo:
                        mt[2, i, rows, :] = jnp.where(lo_s == lo_l, lo, swap(lo)).reshape(PW, 128)
                        return
                    lo_r = swap(lo)
                    hi_r = lo_r if hi is lo else swap(hi)
                    g0, g1 = jnp.where(lo_s, lo, hi_r), jnp.where(lo_s, lo_r, hi)
                    if half:
                        mt[2, i, rows, :] = jnp.where(lo_l, g0, g1).reshape(PW, 128)
                    else:
                        mt[0, i, rows, :] = g0.reshape(PW, 128)
                        mt[1, i, rows, :] = g1.reshape(PW, 128)

                def ld(j):
                    v = (up_s[NT, j, pl.ds(PW * chunk, PW), :] if half else
                         pltpu.bitcast(pool[pl.ds(P_PAR + j * QP + PW * chunk, PW), :], F32))
                    return v.reshape(PW // 8, 8, 128)

                p = {1: (ld(0), ld(1))}
                w = (ld(2), ld(3))
                e = 1
                while e < 1024:
                    p[2 * e] = _csq(p[e])
                    e *= 2
                for i, e in enumerate(MULTS):
                    for part in range(2):
                        put(2 * i + part, p[e][part], p[e][part])
                w1 = _cmul(w, p[1])
                w5 = _cmul(w1, p[4])
                w1032 = _cmul(_cmul(w, p[8]), p[1024])
                w1288 = _cmul(w1032, p[256])
                for i, (u, v) in enumerate(((w1, w5), (w1032, w1288))):
                    put(SEED0 + 2 * i, u[0], v[0])
                    put(SEED0 + 2 * i + 1, -u[1], -v[1])
                put(SEED0 + 4, 1.0, p[8][0])
                put(SEED0 + 5, 0.0, p[8][1])
            yield

    KGEN_STEPS = 3

    def kgen(unit):
        def powers(s):
            ld = lambda i: tuple(mt[s, i + j, pl.ds(pl.multiple_of(8 * unit, 8), 8), :] for j in range(2))
            m = {e: ld(2 * i) for i, e in enumerate(MULTS)}
            mul_conj = lambda x, e: (x[0] * m[e][0] + x[1] * m[e][1], x[1] * m[e][0] - x[0] * m[e][1])
            left = [ld(SEED0)]
            for _ in range(3):
                left.append(mul_conj(left[-1], 1))
            left += [mul_conj(left[1], 256), mul_conj(left[3], 256)]
            for _ in range(2):
                left.append(mul_conj(left[-1], 256))
            left.append(ld(SEED0 + 2))
            left.append(mul_conj(left[-1], 512))
            right = [ld(SEED0 + 4)]
            for _ in range(15):
                right.append(_cmul(right[-1], m[16]))
            return [[jnp.concatenate([_pack_rows(nodes[j][part], nodes[j + 1][part])
                                      for j in range(0, len(nodes), 2)], axis=0) for part in range(2)]
                    for nodes in (left, right)]

        upper = [(re, pltpu.roll(im, 64, 1)) for re, im in powers(2)]
        yield
        for grp in range(2):
            ops = []
            for (re, im), (ure, uim) in zip(powers(grp), upper):
                lo_l = jax.lax.broadcasted_iota(jnp.int32, re.shape, 1) < 64
                top = jnp.where(lo_l, uim, ure) if grp else jnp.where(lo_l, ure, uim)
                ops.append(jnp.concatenate([_to_bf16(v) for v in (re, im, top)], axis=1))
            ko_s[pl.ds((2 * unit + grp) * GP, 80), :] = _dot_nt(*ops)
            yield

    def kgens(first, count):
        return _chain(*[kgen(first + u) for u in range(count)]), count * KGEN_STEPS

    def prep_wqkv(m):
        for i, (r0, nr) in enumerate(((0, 128), (128, 128), (192, 128))):
            wt[i, 0:D, :] = pltpu.bitcast(wraw[m, pl.ds(2 * r0, 2 * nr), :], U32).T
        yield
        for i, (r0, skip) in enumerate(((0, 0), (128, 0), (192, 64))):
            for t in range(NT):
                blk = jnp.concatenate(
                    [wt[i, pl.ds(4 * t + j, H, stride=DH), :] for j in range(4)], axis=0).T
                pool[pool_rows(P_WP + (m * NT + t) * (D // 2) + r0 + skip, 128 - skip), :] = blk[skip:]
            yield

    def prep_wo():
        hi16 = jnp.uint32(0xFFFF0000)
        for c in range(NT):
            wo_w[c, 0:D // 2, :] = pltpu.bitcast(wo_raw[:, 128 * c:128 * (c + 1)], U32)
            for d in range(0, DH, 2):
                even, odd = (wo_w[c, pl.ds(DH // 2 * j + d // 2, H // 2, stride=DH), :] for j in range(2))
                pool[pl.ds(P_WO + c * (D // 2) + H // 2 * d, H), :] = jnp.concatenate(
                    [(even & ~hi16) | (odd << 16), (even >> 16) | (odd & hi16)], axis=0)

    q_scale = float(DH ** -0.5 * np.log2(np.e))

    def project(r0, q_s, k_s, v_s):
        xb = jnp.concatenate([xs[c, pl.ds(r0, RB), :] for c in range(NT)], axis=1)
        dst = [(ref, t, off) for ref, off in ((q_s, 0), (k_s, HALO), (v_s, HALO)) for t in range(NT)]
        for j0 in range(0, 3 * NT, PROJ_TILES):
            js = PROJ_ORDER[j0:j0 + PROJ_TILES]
            w = jnp.concatenate([_to_bf16(pool[pl.ds(P_WP + j * (D // 2), D // 2), :]) for j in js], axis=1)
            y = _dot(xb, w)
            for i, j in enumerate(js):
                ref, t, off = dst[j]
                v = y[:, 128 * i:128 * (i + 1)]
                ref[t, pl.ds(off, RB), :] = v * q_scale if j < NT else v
            yield

    def gate(r0):
        for j in range(RB // 32):
            rows = pl.ds(r0 + 32 * j, 32)
            acc = None
            for c in range(NT):
                xt = xs[c, rows, :]
                io[pool_rows(P_X + c * (S // 2) + r0 // 2 + 16 * j, 16), :] = pltpu.bitcast(xt, U32)
                p = xt.astype(F32) * sd_s[2, pl.ds(c, 1), :]
                acc = p if acc is None else acc + p
            g = jax.nn.sigmoid(jnp.sum(acc, axis=1, keepdims=True))
            io[pool_rows(P_G + r0 + 32 * j, 32), :] = pltpu.bitcast(jnp.broadcast_to(g, (32, 128)), U32)
            yield

    def attend(r0, q_s, k_s, v_s, masked):
        for j in range(RB // 16):
            base = 16 * j
            q = [q_s[t, pl.ds(base, 16), :] for t in range(NT)]
            logits = []
            for w in range(WIN):
                rows = pl.ds(base + HALO - DIL * w, 16)
                s = q[0] * k_s[0, rows, :]
                for t in range(1, NT):
                    s = s + q[t] * k_s[t, rows, :]
                s = s + pltpu.roll(s, 64, 1)
                s = s + pltpu.roll(s, 32, 1)
                if masked and j == 0 and w > 0:
                    pos = r0 + jax.lax.broadcasted_iota(jnp.int32, (16, 128), 0)
                    s = jnp.where(pos >= DIL * w, s, -1e9 * float(np.log2(np.e)))
                logits.append(s)
            yield
            mx = logits[0]
            for s in logits[1:]:
                mx = jnp.maximum(mx, s)
            p = [jnp.exp2(s - mx) for s in logits]
            den = p[0]
            for e in p[1:]:
                den = den + e
            inv = 1.0 / den
            for t in range(NT):
                acc = p[0] * v_s[t, pl.ds(base + HALO, 16), :]
                for w in range(1, WIN):
                    acc = acc + p[w] * v_s[t, pl.ds(base + HALO - DIL * w, 16), :]
                o_s[t, pool_rows(r0 // 2 + base // 2, 8), :] = _to_words(acc * inv)
            yield

    def copy_halo(src, dst):
        for s_ref, d_ref in zip(src, dst):
            for t in range(NT):
                d_ref[t, 0:HALO, :] = s_ref[t, RB:RB + HALO, :]

    uf = (up_s, um_s)

    def x_spectrum(c):
        prev = {}
        for a in range(NB):
            words = pltpu.bitcast(xs[c, pl.ds(CB * a, CB), :], U32)
            xe = pltpu.bitcast(words << 16, F32).astype(BF16)
            xo = pltpu.bitcast(words & jnp.uint32(0xFFFF0000), F32).astype(BF16)
            for odd_f in range(2):
                e, o = (_dot(jnp.concatenate([table(off + 64 * odd_f, 64), table(off + 128 + 64 * odd_f, 64)],
                                             axis=0), v) for off, v in ((OFF_FE, xe), (OFF_FO, xo)))
                for pm, cur in enumerate((e + o, e - o)):
                    re, im = cur[:64], cur[64:]
                    if a:
                        pre, pim = prev[pm, odd_f]
                        re, im = (re + pim, im - pre) if odd_f else (re - pim, im + pre)
                    prev[pm, odd_f] = cur[:64], cur[64:]
                    uf[pm][c, a, pl.ds(64 * odd_f, 64), :] = re
                    uf[pm][c, a, pl.ds(QP + 64 * odd_f, 64), :] = im
            yield

    def k_tile(g0, t):
        src = {a: 16 * (i // 2) + 8 * e + i % 2
               for i, pair in enumerate(A_PAIRS) for e, a in enumerate(pair)}
        slot = (jax.lax.broadcasted_iota(jnp.int32, (32, 128), 1) >> 1) & 3
        parts = []
        for cc in range(4):
            acc = None
            for a4, a in enumerate(K_TILES[t]):
                v = ko_s[pl.ds(g0 * GP + src[a] + 2 * cc, 32, stride=GP), :]
                if a4 != cc:
                    v = pltpu.roll(v, 2 * (a4 - cc) % 128, 1)
                acc = v if acc is None else jnp.where(slot == a4, v, acc)
            parts.append(acc)
        return jnp.concatenate(parts, axis=0)

    def k_samples(c):
        last = jax.lax.broadcasted_iota(jnp.int32, (128, 128), 1) == 127
        tiles = [k_tile(32 * c, t) for t in range(5)]
        tiles += [jnp.where(last, tiles[2], tiles[3]), jnp.where(last, tiles[3], tiles[4])]
        for t, v in enumerate(tiles):
            pool[pl.ds(P_KT + 64 * t, 64), :] = _to_words(v)

    K_TERMS = (((0, 0), (1, 1)), ((2, 1), (3, 2)), ((4, 5),), ((5, 3),), ((6, 6),),
               ((7, 4),), ((8, 4),), ((9, 4),))

    def k_spectrum(c, chunk, out):
        for delta, terms in enumerate(K_TERMS):
            f = jnp.concatenate([table(OFF_K + 512 * i + 128 * chunk, 128) for i, _ in terms], axis=1)
            kt = jnp.concatenate([_to_bf16(pool[pool_rows(P_KT + 64 * t, 64), :])
                                  for _, t in terms], axis=1)
            out.append(_dot_nt(f, kt))
            if delta % 2:
                yield

    def block_products(c, chunk, kf):
        for i in range(4):
            r = 32 * chunk + 8 * i
            for pm in range(2):
                k = [(v[64 * pm + 8 * i:][:8], v[64 * pm + 32 + 8 * i:][:8]) for v in kf]
                k = [(p, q - p, p + q) for p, q in k]
                for outs in PRODUCT_GROUPS:
                    u = [(uf[pm][c, a, pl.ds(r, 8), :], uf[pm][c, a, pl.ds(r + QP, 8), :])
                         for a in range(max(outs) + 1)]
                    u = [(p + q, p, q) for p, q in u]
                    for a in outs:
                        acc = [x * y for x, y in zip(k[0], u[a])]
                        for delta in range(1, a + 1):
                            acc = [z + x * y for x, y, z in zip(k[delta], u[a - delta], acc)]
                        acc = (acc[0] - acc[2], acc[0] + acc[1])
                        uf[pm][NT, a, pl.ds(r, 8), :] = acc[0]
                        uf[pm][NT, a, pl.ds(r + QP, 8), :] = acc[1]
                yield

    def out_proj(c, blocks, out):
        for a in blocks:
            ob = jnp.concatenate([_to_bf16(o_s[t, pl.ds(CB // 2 * a, CB // 2), :]) for t in range(NT)], axis=1)
            out.append(_dot(ob, _to_bf16(pool[pool_rows(P_WO + c * (D // 2), D // 2), :])))
            yield

    def finish(c, att_blocks):
        skip = sd_s[0, pl.ds(c, 1), :]

        def inverse(a):
            yp, ym = (jnp.concatenate([uf[pm][NT, a, pl.ds(QP * j, 128), :] for j in range(2)], axis=0)
                      for pm in range(2))
            for odd in range(2):
                gm = jnp.concatenate([table(OFF_G + 128 * odd, 128),
                                      table(OFF_G + 256 + 128 * odd, 128)], axis=1)
                y_s[a, pl.ds(odd, 128, stride=2), :] = _dot(gm, (yp - ym if odd else yp + ym).astype(BF16))

        def mix(a):
            for j in range(CB // MB):
                r = CB * a + MB * j
                half = c * (S // 2) + r // 2
                b = (y_s[a, pl.ds(MB * j, MB), :]
                     + _to_bf16(io[pool_rows(P_X + half, MB // 2), :]).astype(F32) * skip)
                g = pltpu.bitcast(io[pl.ds(P_G + r, MB), :], F32)
                att = att_blocks[a][MB * j:MB * (j + 1)]
                io[pool_rows(P_OUT + half, MB // 2), :] = _to_words(b + g * (att - b))

        for a in range(NB + MIX_LAG):
            if a < NB:
                inverse(a)
            if a >= MIX_LAG:
                mix(a - MIX_LAG)
                for part, (r0, nr) in enumerate(OUT_PARTS):
                    if r0 + nr == CB * (a - MIX_LAG + 1):
                        out_copy(c, part).start()

    def out_copy(c, part):
        r0, nr = OUT_PARTS[part]
        src = io.bitcast(BF16).at[pl.ds(pl.multiple_of(2 * P_OUT + c * S + r0, CB), nr)]
        dst = out_hbm.at[pl.ds(r0, nr), pl.ds(pl.multiple_of(128 * c, 128), 128)]
        return pltpu.make_async_copy(src, dst, sem_out.at[len(OUT_PARTS) * c + part])

    for cp in p_cp[0] + p_cp[1] + [w_copy(0)]:
        cp.start()
    for c in range(NT):
        row = lambda ref: ref[pl.ds(128 * c, 128)].astype(F32).reshape(1, 128)
        sd_s[0, pl.ds(c, 1), :] = row(dskip_ref)
        sd_s[1, pl.ds(c, 1), :] = jnp.exp(row(ldt_ref)).astype(BF16).astype(F32)
        sd_s[2, pl.ds(c, 1), :] = row(gw_ref)
        for ref in (qb, kb, vb):
            ref[c] = jnp.zeros(ref.shape[1:], F32)

    def prep(c):
        prep_params(c)
        yield
        yield from prep_powers(c)

    for cp in p_cp[0]:
        cp.wait()

    @pl.loop(0, 2)
    def _(c):
        _weave((prep(c), 5))

        @pl.when(c == 0)
        def _():
            for cp in p_cp[1]:
                cp.wait()
            for cp in [x_copy(0), f_cp[0], w_copy(1), x_copy(1)]:
                cp.start()

    for cp in [w_copy(2), x_copy(2), x_copy(3), x_copy(4), wo_cp]:
        cp.start()
    f_cp[0].wait()

    @pl.loop(0, 3)
    def _(m):
        w_copy(m).wait()
        x_copy(m).wait()
        _weave((prep_wqkv(m), 4), (x_spectrum(m), NB))
        _weave((prep(2 + m), 5))

    f_cp[1].start()
    wo_cp.wait()
    prep_wo()
    x_copy(3).wait()
    x_copy(4).wait()
    bufs = ((qa, ka, va), (qb, kb, vb))

    @pl.loop(0, NB)
    def _(a):
        for h in range(2):
            r0 = pl.multiple_of(a * CB + RB * h, RB)
            behind = pl.multiple_of(jnp.maximum(r0 - RB, RB * (1 - h)), RB)
            copy_halo(bufs[1 - h][1:], bufs[h][1:])
            _weave((project(r0, *bufs[h]), 3 * NT // PROJ_TILES),
                   (attend(behind, *bufs[1 - h], h == 1), ATT_STEPS),
                   kgens(2 * UNITS * a + UNITS_1 * h, 2 * UNITS - UNITS_1 if h else UNITS_1), (gate(r0), 4))

    f_cp[1].wait()
    _weave((attend(S - RB, *bufs[1], False), 16), (_chain(x_spectrum(3), x_spectrum(4)), 2 * NB))

    @pl.loop(0, NT)
    def _(c):
        att = []
        _weave((out_proj(c, range(0, OB_AT[0]), att), 1))
        k_samples(c)
        kf = [[] for _ in range(4)]
        _weave((k_spectrum(c, 0, kf[0]), 1))
        for j in range(4):
            blocks = range(OB_AT[j], OB_AT[j + 1])
            streams = [(block_products(c, j, kf[j]), 8), (out_proj(c, blocks, att), max(len(blocks), 1))]
            if j < 3:
                streams.append((k_spectrum(c, j + 1, kf[j + 1]), 4))
            _weave(*streams)
        finish(c, att)

    for c in range(NT):
        for part in range(len(OUT_PARTS)):
            out_copy(c, part).wait()


@jax.jit
def pallas_gated_mix__sliding_local_dilated__ssm_conv_s4__prompt_kernel(
    A_x: jax.Array,
    A_wqkv: jax.Array,
    A_wo: jax.Array,
    B_u: jax.Array,
    B_A_re: jax.Array,
    B_A_im: jax.Array,
    B_B_re: jax.Array,
    B_B_im: jax.Array,
    B_C_re: jax.Array,
    B_C_im: jax.Array,
    B_log_dt: jax.Array,
    B_Dskip: jax.Array,
    gate_w: jax.Array,
):
    del B_u
    hbm = pl.BlockSpec(memory_space=pl.ANY)
    vec = pl.BlockSpec(memory_space=pltpu.VMEM)
    out = pl.pallas_call(
        _kernel,
        out_shape=jax.ShapeDtypeStruct((S, D), BF16),
        in_specs=[hbm] * 9 + [vec] * 3 + [hbm],
        out_specs=hbm,
        scratch_shapes=[
            pltpu.VMEM((NT, S, 128), BF16),
            pltpu.VMEM((P_ROWS, 128), U32),
            pltpu.VMEM((IO_ROWS, 128), U32),
            pltpu.VMEM((NT, S // 2, 128), U32),
            pltpu.VMEM((3, D, D), BF16),
            pltpu.VMEM((D, D), BF16),
            pltpu.VMEM((NT, D // 2 + 24, 128), U32),
            pltpu.VMEM((6, N, D), BF16),
            pltpu.VMEM((3, D + 24, 128), U32),
            pltpu.VMEM((NT, RB, 128), F32),
            pltpu.VMEM((NT, HALO + RB, 128), F32),
            pltpu.VMEM((NT, HALO + RB, 128), F32),
            pltpu.VMEM((NT, RB, 128), F32),
            pltpu.VMEM((NT, HALO + RB, 128), F32),
            pltpu.VMEM((NT, HALO + RB, 128), F32),
            pltpu.VMEM((D // 4 * GP + 96, 128), F32),
            pltpu.VMEM((NT + 1, NB, 2 * QP + 8, 128), F32),
            pltpu.VMEM((NT + 1, NB, 2 * QP + 8, 128), F32),
            pltpu.VMEM((3, 14, D + 8, 128), F32),
            pltpu.VMEM((3, 8, 128), F32),
            pltpu.VMEM((NB, CB + 8, 128), F32),
            pltpu.SemaphoreType.DMA((N_SEMS,)),
            pltpu.SemaphoreType.DMA((3,)),
            pltpu.SemaphoreType.DMA((NT,)),
            pltpu.SemaphoreType.DMA((len(OUT_PARTS) * NT,)),
        ],
        compiler_params=pltpu.CompilerParams(vmem_limit_bytes=100 * 1024 * 1024),
        name="gated_mix",
    )(A_x.reshape(S, D), A_wqkv, A_wo, B_A_re.T, B_A_im.T, B_B_re.T, B_B_im.T, B_C_re.T,
      B_C_im.T, B_log_dt, B_Dskip, gate_w, _F_TABLE)
    return out.reshape(1, S, D)
```
